```python
import jax
import jax.numpy as jnp

def _softmax(x, axis=-1):
    return jax.nn.softmax(x, axis=axis)
def _gelu(x):
    return jax.nn.gelu(x, approximate=True)
def _silu(x):
    return jax.nn.silu(x)
def _sigmoid(x):
    return jax.nn.sigmoid(x)
def _layernorm(x, axis=-1, eps=1e-5):
    m = jnp.mean(x, axis=axis, keepdims=True)
    v = jnp.var(x, axis=axis, keepdims=True)
    return (x - m) / jnp.sqrt(v + eps)
def _scatter_add(tgt, idx, src, axis=0):
    return tgt.at[idx].add(src)
def _segment_sum(src, seg, n):
    return jax.ops.segment_sum(src, seg, n)
class _Rng:
    def __init__(self, key):
        self._k = key
    def _next(self):
        self._k, sub = jax.random.split(self._k)
        return sub
    def normal(self, shape):
        return jax.random.normal(self._next(), shape, dtype=jnp.bfloat16)
    def randint(self, lo, hi, shape):
        return jax.random.randint(self._next(), shape, lo, hi, dtype=jnp.int32)
    def uniform(self, shape, lo=0.0, hi=1.0):
        return jax.random.uniform(self._next(), shape, jnp.bfloat16, lo, hi)
    def permutation(self, n):
        return jax.random.permutation(self._next(), n)


kernel_name = 'gated_mix__mha_block_cached__moe_arch_mod__decode'

def setup_inputs():
    _rng = _Rng(jax.random.key(int.from_bytes(__import__("os").urandom(4), "little")))
    _w = (lambda a: (lambda t: t.astype(jnp.bfloat16) if jnp.issubdtype(t.dtype, jnp.floating) else t)(jnp.asarray(a)))
    def _A_setup():
        B, Sq, D = 4, 1, 1024
        H, Sk, Dh = 32, 8192, 128
        return {
            "x": _w((lambda *s: _rng.normal(s) * 0.05)(B, Sq, D)),
            "k_cache": _w((lambda *s: _rng.normal(s) * 0.05)(B, H, Sk, Dh)),
            "v_cache": _w((lambda *s: _rng.normal(s) * 0.05)(B, H, Sk, Dh)),
            "wq": _w((lambda *s: _rng.normal(s) * 0.05)(D, H * Dh) * (D ** -0.5)),
            "wo": _w((lambda *s: _rng.normal(s) * 0.05)(H * Dh, D) * ((H * Dh) ** -0.5)),
        }
    _A_in = _A_setup()

    def _B_setup():
        B, S, D, F, C = 4, 1, 1024, 3584, 1
        return {
            "x": _w((lambda *s: _rng.normal(s) * 0.05)(B, S, D)),
            "w_r": _w((lambda *s: _rng.normal(s) * 0.05)(D)),
            "w_gate": _w((lambda *s: _rng.normal(s) * 0.05)(D, F)),
            "w_up": _w((lambda *s: _rng.normal(s) * 0.05)(D, F)),
            "w_down": _w((lambda *s: _rng.normal(s) * 0.05)(F, D)),
        }
    _B_in = _B_setup()

    return {
        "A_x": _A_in["x"],
        "A_k_cache": _A_in["k_cache"],
        "A_v_cache": _A_in["v_cache"],
        "A_wq": _A_in["wq"],
        "A_wo": _A_in["wo"],
        "B_x": _B_in["x"],
        "B_w_r": _B_in["w_r"],
        "B_w_gate": _B_in["w_gate"],
        "B_w_up": _B_in["w_up"],
        "B_w_down": _B_in["w_down"],
        "gate_w": _w((lambda *s: _rng.normal(s) * 0.05)(1024)),
    }

def reference(A_x, A_k_cache, A_v_cache, A_wq, A_wo, B_x, B_w_r, B_w_gate, B_w_up, B_w_down, gate_w):
    def _A_ref(x, k_cache, v_cache, wq, wo):
        B, Sq, D = x.shape
        H, Dh = 32, 128
        q = (lambda x, *d: x.transpose(*d))((x @ wq).reshape(B, Sq, H, Dh), 0, 2, 1, 3)
        scores = jnp.einsum("bhqd,bhkd->bhqk", q, k_cache) * (Dh ** -0.5)
        p = _softmax(scores, axis=-1)
        o = jnp.einsum("bhqk,bhkd->bhqd", p, v_cache)
        return (lambda x, *d: x.transpose(*d))(o, 0, 2, 1, 3).reshape(B, Sq, H * Dh) @ wo

    def _B_ref(x, w_r, w_gate, w_up, w_down):
        B, S, D = x.shape
        C = 1
        r = x @ w_r
        idx = jnp.argsort(-r, axis=-1)[:, :C]
        idx_e = jnp.repeat(idx.reshape(B, C, 1), D, axis=2)
        x_sel = jnp.take_along_axis(x, idx_e, axis=1)
        g = _silu(x_sel @ w_gate)
        u = x_sel @ w_up
        y = (g * u) @ w_down
        r_sel = _sigmoid(jnp.take_along_axis(r, idx, axis=1))
        y = y * r_sel.reshape(B, C, 1)
        b_off = (jnp.arange(B) * S).reshape(B, 1)
        flat_idx = (idx + b_off).reshape(B * C)
        zero = (x * 0.0).reshape(B * S, D)
        upd = _scatter_add(zero, flat_idx, y.reshape(B * C, D), axis=0)
        return x + upd.reshape(B, S, D)

    x = A_x
    g = _sigmoid((x * gate_w).sum(-1, keepdims=True))
    a = _A_ref(x, A_k_cache, A_v_cache, A_wq, A_wo)
    b = _B_ref(x, B_w_r, B_w_gate, B_w_up, B_w_down)
    return g * a + (1 - g) * b
```

```python
import jax
import jax.numpy as jnp
import jax.experimental.pallas as pl
import jax.experimental.pallas.tpu as pltpu

B, D = 4, 1024
H, SK, DH = 32, 8192, 128
F = 3584
M = 8

NSLOTS = 4
KV_CHUNK = 192

_NT = (((1,), (1,)), ((), ()))
_NN = (((1,), (0,)), ((), ()))


def _dot(a, b, dims=_NN):
    return jax.lax.dot_general(a, b, dims, preferred_element_type=jnp.float32)


def _sigmoid(x):
    return 1.0 / (1.0 + jnp.exp(-x))


def _row_chunks(n_rows, chunk):
    out, s = [], 0
    while s < n_rows:
        n = min(chunk, n_rows - s)
        out.append((s, n))
        s += n
    return out


def _kernel(x_hbm, k_hbm, v_hbm, wq_hbm, wo_hbm, wr_hbm, wg_hbm, wu_hbm, wd_hbm, gw_hbm,
            o_ref,
            x_buf, wr_buf, gw_buf, wq_buf, wo_buf, wg_buf, wu_buf, wd_buf,
            k_buf, v_buf, q_scr, acc_scr, ffn_scr,
            kv_sems, w_sems):
    n_steps = B * H

    def issue_slab(step, slot):
        h = step // B
        b = step % B
        for s, n in _row_chunks(SK, KV_CHUNK):
            pltpu.make_async_copy(k_hbm.at[b, h, pl.ds(s, n), :], k_buf.at[slot, pl.ds(s, n), :],
                                  kv_sems.at[0, slot]).start(priority=0)
            pltpu.make_async_copy(v_hbm.at[b, h, pl.ds(s, n), :], v_buf.at[slot, pl.ds(s, n), :],
                                  kv_sems.at[1, slot]).start(priority=1)

    def wait_all(buf, sem):
        pltpu.make_async_copy(buf, buf, sem).wait()

    def issue_rows(src, dst, sem, rows_per, n_iter, col_split=False):
        if col_split:
            half = src.shape[1] // 2

            def body(j, c):
                r = pl.multiple_of(j * rows_per, rows_per)
                for t in range(2):
                    pltpu.make_async_copy(src.at[pl.ds(r, rows_per), pl.ds(t * half, half)],
                                          dst.at[pl.ds(r, rows_per), pl.ds(t * half, half)],
                                          sem).start(priority=t)
                return c
        else:
            halfr = src.shape[0] // 2

            def body(j, c):
                for t in range(2):
                    r = pl.multiple_of(t * halfr + j * rows_per, 8)
                    pltpu.make_async_copy(src.at[pl.ds(r, rows_per), :],
                                          dst.at[pl.ds(r, rows_per), :],
                                          sem).start(priority=t)
                return c
        jax.lax.fori_loop(0, n_iter, body, 0)

    small = [
        pltpu.make_async_copy(x_hbm, x_buf, w_sems.at[5]),
        pltpu.make_async_copy(wr_hbm, wr_buf, w_sems.at[6]),
        pltpu.make_async_copy(gw_hbm, gw_buf, w_sems.at[7]),
    ]

    issue_rows(wq_hbm, wq_buf, w_sems.at[0], 8, D // 8, col_split=True)
    for c in small:
        c.start()
    issue_rows(wg_hbm, wg_buf, w_sems.at[2], 8, D // 16)
    issue_rows(wu_hbm, wu_buf, w_sems.at[3], 8, D // 16)
    issue_rows(wd_hbm, wd_buf, w_sems.at[4], 16, F // 32)
    issue_rows(wo_hbm, wo_buf, w_sems.at[1], 16, H * DH // 32)
    for j in range(NSLOTS - 1):
        issue_slab(j, j)

    for c in small:
        c.wait()
    row = jax.lax.broadcasted_iota(jnp.int32, (M, D), 0)
    xf = jnp.zeros((M, D), jnp.float32)
    for b in range(B):
        xb = jnp.broadcast_to(x_buf[b].astype(jnp.float32), (M, D))
        xf = jnp.where(row == b, xb, xf)
    xb16 = xf.astype(jnp.bfloat16)

    wait_all(wq_buf, w_sems.at[0])
    for h in range(H):
        qh = _dot(xb16, wq_buf[:, h * DH:(h + 1) * DH])
        q_scr[h] = qh.astype(jnp.bfloat16).astype(jnp.float32)

    wait_all(wg_buf, w_sems.at[2])
    wait_all(wu_buf, w_sems.at[3])
    hg = _dot(xb16, wg_buf[...])
    hu = _dot(xb16, wu_buf[...])
    hid = (hg * _sigmoid(hg) * hu).astype(jnp.bfloat16)
    wait_all(wd_buf, w_sems.at[4])
    y = _dot(hid, wd_buf[...])
    wr = wr_buf[...].astype(jnp.float32).reshape(1, D)
    gw = gw_buf[...].astype(jnp.float32).reshape(1, D)
    r_sel = _sigmoid(jnp.sum(xf * wr, axis=-1, keepdims=True))
    g = _sigmoid(jnp.sum(xf * gw, axis=-1, keepdims=True))
    b_out = xf + (xf * 0.0 + y * r_sel)
    ffn_scr[0] = (1.0 - g) * b_out
    ffn_scr[1] = jnp.broadcast_to(g, (M, D))
    acc_scr[...] = jnp.zeros_like(acc_scr)
    wait_all(wo_buf, w_sems.at[1])

    scale = DH ** -0.5
    row_o = jax.lax.broadcasted_iota(jnp.int32, (M, DH), 0)

    def step_body(i, c):
        slot = i % NSLOTS
        h = i // B
        b = i % B

        @pl.when(i + NSLOTS - 1 < n_steps)
        def _():
            issue_slab(i + NSLOTS - 1, (i + NSLOTS - 1) % NSLOTS)

        q = q_scr[h].astype(jnp.bfloat16)
        wait_all(k_buf.at[slot], kv_sems.at[0, slot])
        s = _dot(q, k_buf[slot], _NT) * scale
        m = jnp.max(s, axis=-1, keepdims=True)
        p = jnp.exp(s - m)
        l = jnp.sum(p, axis=-1, keepdims=True)
        wait_all(v_buf.at[slot], kv_sems.at[1, slot])
        o = _dot(p.astype(jnp.bfloat16), v_buf[slot])
        o = jnp.where(row_o == b, o / l, 0.0).astype(jnp.bfloat16)
        wo_h = wo_buf[pl.ds(pl.multiple_of(h * DH, DH), DH), :]
        acc_scr[...] += _dot(o, wo_h)
        return c

    jax.lax.fori_loop(0, n_steps, step_body, 0)

    out = ffn_scr[1] * acc_scr[...] + ffn_scr[0]
    for b in range(B):
        o_ref[b] = out[b:b + 1, :].astype(o_ref.dtype)


@jax.jit
def pallas_gated_mix__mha_block_cached__moe_arch_mod__decode_kernel(
    A_x: jax.Array,
    A_k_cache: jax.Array,
    A_v_cache: jax.Array,
    A_wq: jax.Array,
    A_wo: jax.Array,
    B_x: jax.Array,
    B_w_r: jax.Array,
    B_w_gate: jax.Array,
    B_w_up: jax.Array,
    B_w_down: jax.Array,
    gate_w: jax.Array,
):
    del B_x
    bf = jnp.bfloat16
    return pl.pallas_call(
        _kernel,
        in_specs=[pl.BlockSpec(memory_space=pl.ANY)] * 10,
        out_specs=pl.BlockSpec(memory_space=pltpu.VMEM),
        out_shape=jax.ShapeDtypeStruct((B, 1, D), A_x.dtype),
        scratch_shapes=[
            pltpu.VMEM((B, 1, D), bf),
            pltpu.VMEM((D,), bf),
            pltpu.VMEM((D,), bf),
            pltpu.VMEM((D, H * DH), bf),
            pltpu.VMEM((H * DH, D), bf),
            pltpu.VMEM((D, F), bf),
            pltpu.VMEM((D, F), bf),
            pltpu.VMEM((F, D), bf),
            pltpu.VMEM((NSLOTS, SK, DH), bf),
            pltpu.VMEM((NSLOTS, SK, DH), bf),
            pltpu.VMEM((H, M, DH), jnp.float32),
            pltpu.VMEM((M, D), jnp.float32),
            pltpu.VMEM((2, M, D), jnp.float32),
            pltpu.SemaphoreType.DMA((2, NSLOTS)),
            pltpu.SemaphoreType.DMA((8,)),
        ],
        compiler_params=pltpu.CompilerParams(
            vmem_limit_bytes=100 * 1024 * 1024,
            disable_bounds_checks=True,
        ),
    )(A_x, A_k_cache, A_v_cache, A_wq, A_wo, B_w_r, B_w_gate, B_w_up, B_w_down, gate_w)
```

```python
import functools
import jax
import jax.numpy as jnp
import jax.experimental.pallas as pl
import jax.experimental.pallas.tpu as pltpu

B, D = 4, 1024
H, SK, DH = 32, 8192, 128
F = 3584
M = 8
G = 8

_NT = (((1,), (1,)), ((), ()))
_NN = (((1,), (0,)), ((), ()))


def _dot(a, b, dims=_NN):
    return jax.lax.dot_general(a, b, dims, preferred_element_type=jnp.float32)


def _sigmoid(x):
    return 1.0 / (1.0 + jnp.exp(-x))


def make(NSLOTS=2, rows=16, span=1024, tail_segs=2, tail_groups=(7, 1), w_rows=24, compute=True,
         tail_at=0, wq_view=(8, 8, 256), wg_view=(8, 8, 256), wo_view=(8, 8, 256), wd_cols=256, unroll=2,
         weights=True, kv=True, vlag=0):
    J = SK // span
    n_groups = B * H // G
    n_steps = n_groups * J
    HEAD_SEGS = 7 - tail_segs
    assert sum(tail_groups) == tail_segs * 4
    HEAD_ROWS = HEAD_SEGS * 512

    def kernel(x_hbm, k_hbm, v_hbm, wq_hbm, wo_hbm, wr_hbm, wg_hbm, wu_hbm, wd_hbm, gw_hbm,
               o_ref,
               x_buf, wr_buf, gw_buf, wq_buf, wo_buf, wg_buf, wu_buf, wd_buf,
               k_buf, v_buf, q_scr, acc_scr, y_scr, hid_scr, x_scr, gate_scr, m_scr, l_scr, o_scr,
               kv_sems, w_sems, t_sems):

        def loop(n, body):
            def b(j, c):
                body(j)
                return c
            jax.lax.fori_loop(0, n, b, 0, unroll=unroll)

        def issue_slab(step, slot):
            grp = step // J
            base = pl.multiple_of((step % J) * span, span)

            def one(j):
                r = pl.multiple_of(j * rows, rows)
                pltpu.make_async_copy(k_hbm.at[grp, :, pl.ds(base + r, rows), :], k_buf.at[slot, :, pl.ds(r, rows), :],
                                      kv_sems.at[0, slot]).start(priority=0)
                pltpu.make_async_copy(v_hbm.at[grp, :, pl.ds(base + r, rows), :], v_buf.at[slot, :, pl.ds(r, rows), :],
                                      kv_sems.at[1, slot]).start(priority=1)
            loop(span // rows, one)

        def issue_w(src, dst, sem, nseg, rows_, cols):
            _, R, C = src.shape
            ncb = C // cols
            halfr = R // 2
            n = (halfr // rows_) * ncb

            def one(j):
                rb = j // ncb
                cb = j % ncb
                c = pl.multiple_of(cb * cols, 128)
                for t in range(2):
                    r = pl.multiple_of(t * halfr + rb * rows_, 8)
                    pltpu.make_async_copy(src.at[pl.ds(0, nseg), pl.ds(r, rows_), pl.ds(c, cols)],
                                          dst.at[pl.ds(0, nseg), pl.ds(r, rows_), pl.ds(c, cols)], sem).start(priority=t)
            loop(n, one)

        def wait_all(buf, sem):
            pltpu.make_async_copy(buf, buf, sem).wait()

        small = [
            pltpu.make_async_copy(x_hbm, x_buf, w_sems.at[5]),
            pltpu.make_async_copy(wr_hbm, wr_buf, w_sems.at[6]),
            pltpu.make_async_copy(gw_hbm, gw_buf, w_sems.at[7]),
        ]

        gl = []
        blk = HEAD_SEGS * 4
        for gsz in tail_groups:
            gl.append(list(range(blk, blk + gsz)))
            blk += gsz

        def issue_tail():
            for j, blks in enumerate(gl):
                for bk in blks:
                    seg, r0 = bk // 4, (bk % 4) * 128
                    for s in range(0, 64, w_rows):
                        n = min(w_rows, 64 - s)
                        for t in range(2):
                            r = r0 + t * 64 + s
                            pltpu.make_async_copy(wd_hbm.at[seg, pl.ds(r, n), :], wd_buf.at[seg, pl.ds(r, n), :],
                                                  t_sems.at[j]).start(priority=t)

        def wait_tail(j):
            for bk in gl[j]:
                seg, r0 = bk // 4, (bk % 4) * 128
                wait_all(wd_buf.at[seg, pl.ds(r0, 128), :], t_sems.at[j])

        if weights:
            issue_w(wq_hbm, wq_buf, w_sems.at[0], *wq_view)
        for c in small:
            c.start()
        if weights:
            issue_w(wg_hbm, wg_buf, w_sems.at[2], *wg_view)

        for c in small:
            c.wait()
        xf = jnp.concatenate([x_buf[...].astype(jnp.float32), jnp.zeros((M - B, D), jnp.float32)], axis=0)
        x_scr[...] = xf

        def colmm(w_buf, cb, store):
            S, R, C = w_buf.shape

            def body(j, c):
                c0 = pl.multiple_of(j * cb, 128)
                w = w_buf[:, :, pl.ds(c0, cb)].reshape(S * R, cb)
                store(j, c0, _dot(x_scr[...].astype(jnp.bfloat16), w))
                return c
            jax.lax.fori_loop(0, C // cb, body, 0)

        if weights:
            wait_all(wq_buf, w_sems.at[0])
        if compute:
            def st_q(j, c0, r):
                r = r.astype(jnp.bfloat16).astype(jnp.float32)
                for b in range(B):
                    for t in range(4):
                        q_scr[pl.ds(b * H + j * 4 + t, 1), :] = r[b:b + 1, t * DH:(t + 1) * DH]
            colmm(wq_buf, 512, st_q)

        if weights:
            issue_w(wu_hbm, wu_buf, w_sems.at[3], *wg_view)
            wait_all(wg_buf, w_sems.at[2])
        if compute:
            def st_g(j, c0, r):
                hid_scr[:, pl.ds(c0, 512)] = r * _sigmoid(r)
            colmm(wg_buf, 512, st_g)
        if weights:
            issue_w(wd_hbm, wd_buf, w_sems.at[4], HEAD_SEGS, 8, wd_cols)
            wait_all(wu_buf, w_sems.at[3])
        if compute:
            def st_u(j, c0, r):
                hid_scr[:, pl.ds(c0, 512)] = hid_scr[:, pl.ds(c0, 512)] * r
            colmm(wu_buf, 512, st_u)
        if weights:
            issue_w(wo_hbm, wo_buf, w_sems.at[1], *wo_view)
            wait_all(wd_buf.at[pl.ds(0, HEAD_SEGS)], w_sems.at[4])
        y_scr[...] = jnp.zeros_like(y_scr)
        if compute:
            def dbody(j, c):
                r0 = pl.multiple_of(j * 512, 512)
                y_scr[...] += _dot(hid_scr[:, pl.ds(r0, 512)].astype(jnp.bfloat16), wd_buf[j])
                return c
            jax.lax.fori_loop(0, HEAD_SEGS, dbody, 0)
        wr = wr_buf[...].astype(jnp.float32).reshape(1, D)
        gw = gw_buf[...].astype(jnp.float32).reshape(1, D)
        r_sel = _sigmoid(jnp.sum(xf * wr, axis=-1, keepdims=True))
        g = _sigmoid(jnp.sum(xf * gw, axis=-1, keepdims=True))
        gate_scr[0] = jnp.broadcast_to(g, (M, D))
        gate_scr[1] = jnp.broadcast_to((1.0 - g) * r_sel, (M, D))
        gate_scr[2] = (1.0 - g) * (xf + xf * 0.0)
        acc_scr[...] = jnp.zeros_like(acc_scr)
        if kv:
            for j in range(NSLOTS - 1):
                issue_slab(j, j)
        if weights:
            wait_all(wo_buf, w_sems.at[1])

        scale = DH ** -0.5
        row_s = jax.lax.broadcasted_iota(jnp.int32, (M, span), 0)
        row_o = jax.lax.broadcasted_iota(jnp.int32, (M, DH), 0)
        row_d = jax.lax.broadcasted_iota(jnp.int32, (M, D), 0)
        col_d = jax.lax.broadcasted_iota(jnp.int32, (M, D), 1)

        def step_body(i, c):
            slot = i % NSLOTS
            grp = i // J
            jj = i % J

            if kv:
                @pl.when(i + NSLOTS - 1 < n_steps)
                def _():
                    issue_slab(i + NSLOTS - 1, (i + NSLOTS - 1) % NSLOTS)

            if weights:
                @pl.when(i == n_steps - 1 - tail_at)
                def _():
                    issue_tail()

            @pl.when(jj == 0)
            def _():
                m_scr[...] = jnp.full_like(m_scr, -jnp.inf)
                l_scr[...] = jnp.zeros_like(l_scr)
                o_scr[...] = jnp.zeros_like(o_scr)

            if kv:
                wait_all(k_buf.at[slot], kv_sems.at[0, slot])
            if compute:
                q = q_scr[pl.ds(pl.multiple_of(grp * G, G), G), :].astype(jnp.bfloat16)
                s = _dot(q, k_buf[slot, 0], _NT)
                for h in range(1, G):
                    s = jnp.where(row_s == h, _dot(q, k_buf[slot, h], _NT), s)
                s = s * scale
                m_old = m_scr[...]
                m_new = jnp.maximum(m_old, jnp.max(s, axis=-1, keepdims=True))
                alpha = jnp.exp(m_old - m_new)
                p = jnp.exp(s - m_new[:, :1])
                l_scr[...] = l_scr[...] * alpha + jnp.sum(p, axis=-1, keepdims=True)
                m_scr[...] = m_new
                pb = p.astype(jnp.bfloat16)
            if kv:
                wait_all(v_buf.at[slot], kv_sems.at[1, slot])
            if compute:
                o = _dot(pb, v_buf[slot, 0])
                for h in range(1, G):
                    o = jnp.where(row_o == h, _dot(pb, v_buf[slot, h]), o)
                o_scr[...] = o_scr[...] * alpha + o

                @pl.when(jj == J - 1)
                def _():
                    on = o_scr[...] / l_scr[...]
                    obd = jnp.where(col_d // DH == row_d, jnp.concatenate([on] * G, axis=1), 0.0).astype(jnp.bfloat16)
                    hg = grp % (H // G)
                    w = wo_buf[pl.ds(hg * 2, 2)].reshape(G * DH, D)
                    a = jnp.sum(_dot(obd, w), axis=0, keepdims=True)
                    bb = grp // (H // G)
                    acc_scr[...] += jnp.where(row_d == bb, a, 0.0)
            return c

        jax.lax.fori_loop(0, n_steps, step_body, 0)

        base = gate_scr[0] * acc_scr[...] + gate_scr[2]
        y = y_scr[...]
        for j, blks in enumerate(gl):
            if weights:
                wait_tail(j)
            if compute:
                for bk in blks:
                    seg, r0 = bk // 4, (bk % 4) * 128
                    y = y + _dot(hid_scr[:, bk * 128:(bk + 1) * 128].astype(jnp.bfloat16), wd_buf[seg, pl.ds(r0, 128), :])
        out = base + gate_scr[1] * y
        o_ref[...] = out[:B].astype(o_ref.dtype)

    @jax.jit
    def fn(A_x, A_k_cache, A_v_cache, A_wq, A_wo, B_x, B_w_r, B_w_gate, B_w_up, B_w_down, gate_w):
        bf = jnp.bfloat16
        wq = A_wq.reshape(wq_view[0], D // wq_view[0], H * DH)
        wg = B_w_gate.reshape(wg_view[0], D // wg_view[0], F)
        wu = B_w_up.reshape(wg_view[0], D // wg_view[0], F)
        wo = A_wo.reshape(8, 512, D)
        wd = B_w_down.reshape(7, 512, D)
        out = pl.pallas_call(
            kernel,
            in_specs=[pl.BlockSpec(memory_space=pl.ANY)] * 10,
            out_specs=pl.BlockSpec(memory_space=pltpu.VMEM),
            out_shape=jax.ShapeDtypeStruct((B, D), A_x.dtype),
            scratch_shapes=[
                pltpu.VMEM((B, D), bf),
                pltpu.VMEM((D,), bf),
                pltpu.VMEM((D,), bf),
                pltpu.VMEM(wq.shape, bf),
                pltpu.VMEM(wo.shape, bf),
                pltpu.VMEM(wg.shape, bf),
                pltpu.VMEM(wu.shape, bf),
                pltpu.VMEM(wd.shape, bf),
                pltpu.VMEM((NSLOTS, G, span, DH), bf),
                pltpu.VMEM((NSLOTS, G, span, DH), bf),
                pltpu.VMEM((B * H, DH), jnp.float32),
                pltpu.VMEM((M, D), jnp.float32),
                pltpu.VMEM((M, D), jnp.float32),
                pltpu.VMEM((M, F), jnp.float32),
                pltpu.VMEM((M, D), jnp.float32),
                pltpu.VMEM((3, M, D), jnp.float32),
                pltpu.VMEM((M, DH), jnp.float32),
                pltpu.VMEM((M, DH), jnp.float32),
                pltpu.VMEM((M, DH), jnp.float32),
                pltpu.SemaphoreType.DMA((2, NSLOTS)),
                pltpu.SemaphoreType.DMA((8,)),
                pltpu.SemaphoreType.DMA((max(len(tail_groups), 1),)),
            ],
            compiler_params=pltpu.CompilerParams(
                vmem_limit_bytes=100 * 1024 * 1024,
                disable_bounds_checks=True,
                disable_semaphore_checks=True,
            ),
        )(A_x.reshape(B, D), A_k_cache.reshape(n_groups, G, SK, DH), A_v_cache.reshape(n_groups, G, SK, DH),
          wq, wo, B_w_r, wg, wu, wd, gate_w)
        return out.reshape(B, 1, D)
    return fn


_IMPL = make()


@jax.jit
def pallas_gated_mix__mha_block_cached__moe_arch_mod__decode_kernel(
    A_x: jax.Array,
    A_k_cache: jax.Array,
    A_v_cache: jax.Array,
    A_wq: jax.Array,
    A_wo: jax.Array,
    B_x: jax.Array,
    B_w_r: jax.Array,
    B_w_gate: jax.Array,
    B_w_up: jax.Array,
    B_w_down: jax.Array,
    gate_w: jax.Array,
):
    return _IMPL(A_x, A_k_cache, A_v_cache, A_wq, A_wo, B_x, B_w_r, B_w_gate, B_w_up, B_w_down, gate_w)
```

```python
import functools
import jax
import jax.numpy as jnp
import jax.experimental.pallas as pl
import jax.experimental.pallas.tpu as pltpu

B, D = 4, 1024
H, SK, DH = 32, 8192, 128
F = 3584
M = 8
G = 8
NSEG_D, SEG_D = 7, 512
WC = 256

_NT = (((1,), (1,)), ((), ()))
_NN = (((1,), (0,)), ((), ()))


def _dot(a, b, dims=_NN):
    return jax.lax.dot_general(a, b, dims, preferred_element_type=jnp.float32)


def _sigmoid(x):
    return 1.0 / (1.0 + jnp.exp(-x))


def make(NV=2, DSH=3, compute=True, hs=1, kth=1, lead=26, last_cols=(512, 256, 128, 128), bursts=(96, 62, 62), unroll=2,
         c_loop=True, c_tail=True, npoll=0, qth=0, gth=0, wd_split="half", gu_burst=48, solo=0, lead_b=0):
    rows, span = 16, 1024
    ND = span // rows
    NK = NV + DSH
    J = SK // span
    n_groups = B * H // G
    n_steps = n_groups * J
    assert sum(last_cols) == D and lead % 2 == 0 and 0 < DSH < J
    tK, tV = kth, 1 - kth
    AH = NV - 1 + DSH
    n_gu = D // 64 * (F // WC)
    assert AH * gu_burst <= n_gu

    def kernel(x_hbm, k_hbm, v_hbm, wq_hbm, wo_hbm, wr_hbm, wg_hbm, wu_hbm, wd_hbm, gw_hbm,
               o_ref, *rest):
        if npoll:
            dbg_ref, rest = rest[0], rest[1:]
        (x_buf, wr_buf, gw_buf, wq_buf, wo_buf, wg_buf, wu_buf, wd_buf,
         k_buf, v_buf, q_scr, acc_scr, hid_scr, x_scr, st_scr, sv_scr,
         k_sems, v_sems, w_sems, d_sems) = rest

        def mo(x, m):
            return x if isinstance(x, int) else pl.multiple_of(x, m)

        def kv_stream(hbm, buf, sems, blk, slot):
            grp = blk // J
            go, gi = grp // hs, grp % hs
            base = mo((blk % J) * span, span)

            def f(j):
                r = mo(j * rows, rows)
                return pltpu.make_async_copy(hbm.at[go, :, gi, pl.ds(base + r, rows), :],
                                             buf.at[slot, :, pl.ds(r, rows), :], sems.at[slot])
            return f

        def v_slot(blk):
            if isinstance(blk, int):
                return NV + blk if blk < DSH else blk % NV
            return jnp.where(blk < DSH, NV + blk, blk % NV)

        def w_stream(src, dst, sem, off=0):
            ncb = src.shape[2] // WC

            def f(j):
                j = j + off
                r = mo((j // ncb) * 8, 8)
                c = mo((j % ncb) * WC, 128)
                return pltpu.make_async_copy(src.at[:, pl.ds(r, 8), pl.ds(c, WC)],
                                             dst.at[:, pl.ds(r, 8), pl.ds(c, WC)], sem)
            return f

        def shifted(f, off):
            return lambda j: f(j + off)

        def issue(fa, fb, n, ta):
            def b(j, c):
                fa(j).start(priority=ta)
                fb(j).start(priority=1 - ta)
                return c
            jax.lax.fori_loop(0, n, b, 0, unroll=unroll if n % unroll == 0 else 1)

        def issue_kv(u):
            issue(kv_stream(k_hbm, k_buf, k_sems, (u + DSH) % n_steps, u % NK),
                  kv_stream(v_hbm, v_buf, v_sems, u, v_slot(u)), ND, tK)

        def wait_all(buf, sem):
            pltpu.make_async_copy(buf, buf, sem).wait()

        wq_s = w_stream(wq_hbm, wq_buf, w_sems.at[0])
        wo_s = w_stream(wo_hbm, wo_buf, w_sems.at[1])
        wg_s = w_stream(wg_hbm, wg_buf, w_sems.at[2])
        wu_s = w_stream(wu_hbm, wu_buf, w_sems.at[3])

        small = [
            pltpu.make_async_copy(x_hbm, x_buf, w_sems.at[4]),
            pltpu.make_async_copy(wr_hbm, wr_buf, w_sems.at[5]),
            pltpu.make_async_copy(gw_hbm, gw_buf, w_sems.at[6]),
        ]

        batches = [(0, 0, 0, D), (1, 128, 0, D), (2, 256, 0, D)]
        c0 = 0
        for t, nc in enumerate(last_cols):
            batches.append((3 + t, 384, c0, nc))
            c0 += nc
        L = [[], []]
        for bi, (si, r0, c0, nc) in enumerate(batches):
            w = min(WC, nc)
            assert nc % w == 0
            ds = [(r, c, w, si) for r in range(r0, r0 + 128, 8) for c in range(c0, c0 + nc, w)]
            n0 = len(ds) // 2 + (lead // 2 if bi == lead_b else 0)
            if bi >= len(batches) - solo:
                n0 = 0
            L[0] += ds[:n0]
            L[1] += ds[n0:]
        seq = []
        for j in range(max(len(L[0]), len(L[1]))):
            for t in (1, 0):
                if j < len(L[t]):
                    seq.append((t, L[t][j]))

        def issue_seq(lo, hi):
            for t, (r, c, w, si) in seq[lo:hi]:
                pltpu.make_async_copy(wd_hbm.at[:, pl.ds(r, 8), pl.ds(c, w)], wd_buf.at[:, pl.ds(r, 8), pl.ds(c, w)],
                                      d_sems.at[si]).start(priority=t)

        issue(wq_s, wo_s, 32, qth)
        for c in small:
            c.start()
        issue(shifted(wq_s, 32), shifted(wo_s, 32), 256 - 32, qth)
        issue_kv(0)

        for c in small:
            c.wait()
        x_scr[...] = jnp.concatenate([x_buf[...].astype(jnp.float32), jnp.zeros((M - B, D), jnp.float32)], axis=0)

        def colmm(w_buf, cb, store):
            S, R, C = w_buf.shape

            def body(j, c):
                c0 = pl.multiple_of(j * cb, 128)
                w = w_buf[:, :, pl.ds(c0, cb)].reshape(S * R, cb)
                store(j, c0, _dot(x_scr[...].astype(jnp.bfloat16), w))
                return c
            jax.lax.fori_loop(0, C // cb, body, 0)

        wait_all(wq_buf, w_sems.at[0])
        if compute:
            def st_q(j, c0, r):
                r = r.astype(jnp.bfloat16).astype(jnp.float32)
                for b in range(B):
                    for t in range(4):
                        h = j * 4 + t
                        if hs == 1:
                            row = b * H + h
                        else:
                            ho = h // (G * hs)
                            rem = h % (G * hs)
                            row = b * H + ho * (G * hs) + (rem % hs) * G + rem // hs
                        q_scr[pl.ds(row, 1), :] = r[b:b + 1, t * DH:(t + 1) * DH]
            colmm(wq_buf, 512, st_q)
        acc_scr[...] = jnp.zeros_like(acc_scr)

        def pre(u, c):
            issue_kv(u)
            return c
        jax.lax.fori_loop(1, AH, pre, 0)
        wait_all(wo_buf, w_sems.at[1])

        scale = DH ** -0.5
        row_s = jax.lax.broadcasted_iota(jnp.int32, (M, span), 0)
        row_o = jax.lax.broadcasted_iota(jnp.int32, (M, DH), 0)
        row_d = jax.lax.broadcasted_iota(jnp.int32, (M, D), 0)
        col_d = jax.lax.broadcasted_iota(jnp.int32, (M, D), 1)

        def step_body(t, c):
            blk = (t + DSH) % n_steps
            kslot = t % NK
            vslot = v_slot(blk)
            grp = blk // J
            jj = blk % J
            u = t + AH

            @pl.when(u < n_steps)
            def _():
                issue_kv(u)

            @pl.when(u >= n_steps)
            def _():
                off = (u - n_steps) * gu_burst
                issue(shifted(wg_s, off), shifted(wu_s, off), gu_burst, gth)

            resume = t == n_steps - DSH

            @pl.when(jnp.logical_or(t == 0, jnp.logical_and(jj == 0, jnp.logical_not(resume))))
            def _():
                st_scr[0] = jnp.full((M, DH), -jnp.inf, jnp.float32)
                st_scr[1] = jnp.zeros((M, DH), jnp.float32)
                st_scr[2] = jnp.zeros((M, DH), jnp.float32)

            @pl.when(resume)
            def _():
                st_scr[...] = sv_scr[...]

            wait_all(k_buf.at[kslot], k_sems.at[kslot])
            if compute and c_loop:
                q = q_scr[pl.ds(pl.multiple_of(grp * G, G), G), :].astype(jnp.bfloat16)
                s = _dot(q, k_buf[kslot, 0], _NT)
                for h in range(1, G):
                    s = jnp.where(row_s == h, _dot(q, k_buf[kslot, h], _NT), s)
                s = s * scale
                m_old = st_scr[0]
                m_new = jnp.maximum(m_old, jnp.max(s, axis=-1, keepdims=True))
                alpha = jnp.exp(m_old - m_new)
                p = jnp.exp(s - m_new[:, :1])
                st_scr[1] = st_scr[1] * alpha + jnp.sum(p, axis=-1, keepdims=True)
                st_scr[0] = m_new
                pb = p.astype(jnp.bfloat16)
            wait_all(v_buf.at[vslot], v_sems.at[vslot])
            if compute and c_loop:
                o = _dot(pb, v_buf[vslot, 0])
                for h in range(1, G):
                    o = jnp.where(row_o == h, _dot(pb, v_buf[vslot, h]), o)
                st_scr[2] = st_scr[2] * alpha + o

            suspend = t == J - 1 - DSH

            @pl.when(suspend)
            def _():
                sv_scr[...] = st_scr[...]

            if compute and c_loop:
                @pl.when(jnp.logical_or(t == n_steps - 1, jnp.logical_and(jj == J - 1, jnp.logical_not(suspend))))
                def _():
                    on = st_scr[2] / st_scr[1]
                    gpb = H // G
                    bb = grp // gpb
                    hg = grp % gpb
                    if hs == 1:
                        obd = jnp.where(col_d // DH == row_d, jnp.concatenate([on] * G, axis=1), 0.0).astype(jnp.bfloat16)
                        w = wo_buf[pl.ds(hg * 2, 2)].reshape(G * DH, D)
                        a = jnp.sum(_dot(obd, w), axis=0, keepdims=True)
                    else:
                        ho = hg // hs
                        gi = hg % hs
                        a8 = jnp.zeros((M, D), jnp.float32)
                        for g in range(G):
                            h = ho * (G * hs) + g * hs + gi
                            w = wo_buf[h // 4, pl.ds(pl.multiple_of((h % 4) * DH, DH), DH), :]
                            a8 = a8 + _dot(jnp.where(row_o == g, on, 0.0).astype(jnp.bfloat16), w)
                        a = jnp.sum(a8, axis=0, keepdims=True)
                    acc_scr[...] += jnp.where(row_d == bb, a, 0.0)
            return c

        jax.lax.fori_loop(0, n_steps, step_body, 0)

        ct = compute and c_tail
        done = AH * gu_burst
        if n_gu > done:
            issue(shifted(wg_s, done), shifted(wu_s, done), n_gu - done, gth)
        b1, b2, b3 = bursts[0], bursts[0] + bursts[1], sum(bursts)
        issue_seq(0, b1)
        wait_all(wg_buf, w_sems.at[2])
        if ct:
            def st_g(j, c0, r):
                hid_scr[:, pl.ds(c0, 512)] = r * _sigmoid(r)
            colmm(wg_buf, 512, st_g)
        issue_seq(b1, b2)
        wait_all(wu_buf, w_sems.at[3])
        if ct:
            def st_u(j, c0, r):
                hid_scr[:, pl.ds(c0, 512)] = hid_scr[:, pl.ds(c0, 512)] * r
            colmm(wu_buf, 512, st_u)
        issue_seq(b2, b3)

        xf = x_scr[...]
        wr = wr_buf[...].astype(jnp.float32).reshape(1, D)
        gw = gw_buf[...].astype(jnp.float32).reshape(1, D)
        r_sel = _sigmoid(jnp.sum(xf * wr, axis=-1, keepdims=True))
        g = _sigmoid(jnp.sum(xf * gw, axis=-1, keepdims=True))
        base = g * acc_scr[...] + (1.0 - g) * (xf + xf * 0.0)
        coef = (1.0 - g) * r_sel

        def down(piece, c0, nc):
            r0 = piece * 128
            y = None
            for sg in range(NSEG_D):
                lo = sg * SEG_D + r0
                t = _dot(hid_scr[:, lo:lo + 128].astype(jnp.bfloat16), wd_buf[sg, r0:r0 + 128, c0:c0 + nc])
                y = t if y is None else y + t
            return y

        y = jnp.zeros((M, D), jnp.float32)
        for p in range(3):
            if npoll and p == 2:
                def poll(j, c):
                    for t in range(1 + len(last_cols)):
                        dbg_ref[t, j] = pl.semaphore_read(d_sems.at[2 + t])
                    return c
                jax.lax.fori_loop(0, npoll, poll, 0)
            wait_all(wd_buf.at[:, pl.ds(p * 128, 128), :], d_sems.at[p])
            if ct:
                y = y + down(p, 0, D)
            if p == 0:
                issue_seq(b3, len(seq))
        c0 = 0
        for t, nc in enumerate(last_cols):
            wait_all(wd_buf.at[:, pl.ds(384, 128), pl.ds(c0, nc)], d_sems.at[3 + t])
            yc = y[:, c0:c0 + nc]
            if ct:
                yc = yc + down(3, c0, nc)
            o_ref[:, c0:c0 + nc] = (base[:, c0:c0 + nc] + coef * yc)[:B].astype(o_ref.dtype)
            c0 += nc

    @jax.jit
    def fn(A_x, A_k_cache, A_v_cache, A_wq, A_wo, B_x, B_w_r, B_w_gate, B_w_up, B_w_down, gate_w):
        bf = jnp.bfloat16
        wq = A_wq.reshape(8, D // 8, H * DH)
        wg = B_w_gate.reshape(8, D // 8, F)
        wu = B_w_up.reshape(8, D // 8, F)
        wo = A_wo.reshape(8, 512, D)
        wd = B_w_down.reshape(NSEG_D, SEG_D, D)
        kv_shape = (n_groups // hs, G, hs, SK, DH)
        out_specs = pl.BlockSpec(memory_space=pltpu.VMEM)
        out_shape = jax.ShapeDtypeStruct((B, D), A_x.dtype)
        if npoll:
            out_specs = [out_specs, pl.BlockSpec(memory_space=pltpu.SMEM)]
            out_shape = [out_shape, jax.ShapeDtypeStruct((1 + len(last_cols), npoll), jnp.int32)]
        out = pl.pallas_call(
            kernel,
            in_specs=[pl.BlockSpec(memory_space=pl.ANY)] * 10,
            out_specs=out_specs,
            out_shape=out_shape,
            scratch_shapes=[
                pltpu.VMEM((B, D), bf),
                pltpu.VMEM((D,), bf),
                pltpu.VMEM((D,), bf),
                pltpu.VMEM(wq.shape, bf),
                pltpu.VMEM(wo.shape, bf),
                pltpu.VMEM(wg.shape, bf),
                pltpu.VMEM(wu.shape, bf),
                pltpu.VMEM(wd.shape, bf),
                pltpu.VMEM((NK, G, span, DH), bf),
                pltpu.VMEM((NV + DSH, G, span, DH), bf),
                pltpu.VMEM((B * H, DH), jnp.float32),
                pltpu.VMEM((M, D), jnp.float32),
                pltpu.VMEM((M, F), jnp.float32),
                pltpu.VMEM((M, D), jnp.float32),
                pltpu.VMEM((3, M, DH), jnp.float32),
                pltpu.VMEM((3, M, DH), jnp.float32),
                pltpu.SemaphoreType.DMA((NK,)),
                pltpu.SemaphoreType.DMA((NV + DSH,)),
                pltpu.SemaphoreType.DMA((7,)),
                pltpu.SemaphoreType.DMA((3 + len(last_cols),)),
            ],
            compiler_params=pltpu.CompilerParams(
                vmem_limit_bytes=100 * 1024 * 1024,
                disable_bounds_checks=True,
                disable_semaphore_checks=True,
            ),
        )(A_x.reshape(B, D), A_k_cache.reshape(kv_shape), A_v_cache.reshape(kv_shape),
          wq, wo, B_w_r, wg, wu, wd, gate_w)
        if npoll:
            return out[1]
        return out.reshape(B, 1, D)
    return fn


_IMPL = make(NV=3, gu_burst=40, solo=2, lead=26, last_cols=(768, 128, 128))


@jax.jit
def pallas_gated_mix__mha_block_cached__moe_arch_mod__decode_kernel(
    A_x: jax.Array,
    A_k_cache: jax.Array,
    A_v_cache: jax.Array,
    A_wq: jax.Array,
    A_wo: jax.Array,
    B_x: jax.Array,
    B_w_r: jax.Array,
    B_w_gate: jax.Array,
    B_w_up: jax.Array,
    B_w_down: jax.Array,
    gate_w: jax.Array,
):
    return _IMPL(A_x, A_k_cache, A_v_cache, A_wq, A_wo, B_x, B_w_r, B_w_gate, B_w_up, B_w_down, gate_w)
```

```python
import jax
import jax.numpy as jnp
import jax.experimental.pallas as pl
import jax.experimental.pallas.tpu as pltpu

M = 8
G = 8
ROWS = 16
SPAN = 1024
NV = 3
DSH = 3
K_THREAD = 1
WSEG = 8
WC = 256
SEG_D = 512
GU_BURST = 40
LEAD = 26
LAST_COLS = (768, 128, 128)
SOLO = 2
BURSTS = (96, 62, 62)
UNROLL = 2

_NT = (((1,), (1,)), ((), ()))
_NN = (((1,), (0,)), ((), ()))


def _dot(a, b, dims=_NN):
    return jax.lax.dot_general(a, b, dims, preferred_element_type=jnp.float32)


def _sigmoid(x):
    return 1.0 / (1.0 + jnp.exp(-x))


def _mo(x, m):
    return x if isinstance(x, int) else pl.multiple_of(x, m)


def _w_down_schedule(d):
    batches = [(p, p * 128, 0, d) for p in range(3)]
    c0 = 0
    for t, nc in enumerate(LAST_COLS):
        batches.append((3 + t, 384, c0, nc))
        c0 += nc
    assert c0 == d
    lists = [[], []]
    for bi, (si, r0, c0, nc) in enumerate(batches):
        w = min(WC, nc)
        assert nc % w == 0
        ds = [(r, c, w, si) for r in range(r0, r0 + 128, 8) for c in range(c0, c0 + nc, w)]
        n0 = len(ds) // 2 + (LEAD // 2 if bi == 0 else 0)
        if bi >= len(batches) - SOLO:
            n0 = 0
        lists[0] += ds[:n0]
        lists[1] += ds[n0:]
    seq = []
    for j in range(max(len(lists[0]), len(lists[1]))):
        for t in (1, 0):
            if j < len(lists[t]):
                seq.append((t,) + lists[t][j])
    return seq


def _kernel(x_hbm, k_hbm, v_hbm, wq_hbm, wo_hbm, wr_hbm, wg_hbm, wu_hbm, wd_hbm, gw_hbm,
            o_ref,
            x_buf, wr_buf, gw_buf, wq_buf, wo_buf, wg_buf, wu_buf, wd_buf,
            k_buf, v_buf, q_scr, acc_scr, hid_scr, x_scr, st_scr, sv_scr,
            k_sems, v_sems, w_sems, d_sems):
    B, D = x_buf.shape
    n_groups, _, SK, DH = k_hbm.shape
    H = n_groups * G // B
    span = k_buf.shape[2]
    nseg_d = wd_buf.shape[0]
    NK = NV + DSH
    AH = NV - 1 + DSH
    ND = span // ROWS
    J = SK // span
    n_steps = n_groups * J
    n_qo = wq_buf.shape[1] // 8 * (wq_buf.shape[2] // WC)
    n_gu = wg_buf.shape[1] // 8 * (wg_buf.shape[2] // WC)
    assert n_qo == wo_buf.shape[1] // 8 * (wo_buf.shape[2] // WC)
    assert 0 < DSH < J and AH * GU_BURST <= n_gu and wd_buf.shape[1] == 512

    def kv_stream(hbm, buf, sems, blk, slot):
        grp = blk // J
        base = _mo((blk % J) * span, span)

        def f(j):
            r = _mo(j * ROWS, ROWS)
            return pltpu.make_async_copy(hbm.at[grp, :, pl.ds(base + r, ROWS), :],
                                         buf.at[slot, :, pl.ds(r, ROWS), :], sems.at[slot])
        return f

    def v_slot(blk):
        if isinstance(blk, int):
            return NV + blk if blk < DSH else blk % NV
        return jnp.where(blk < DSH, NV + blk, blk % NV)

    def w_stream(src, dst, sem, off):
        ncb = src.shape[2] // WC

        def f(j):
            j = j + off
            r = _mo((j // ncb) * 8, 8)
            c = _mo((j % ncb) * WC, 128)
            return pltpu.make_async_copy(src.at[:, pl.ds(r, 8), pl.ds(c, WC)],
                                         dst.at[:, pl.ds(r, 8), pl.ds(c, WC)], sem)
        return f

    def issue(fa, fb, n, thread_a):
        def body(j, c):
            fa(j).start(priority=thread_a)
            fb(j).start(priority=1 - thread_a)
            return c
        jax.lax.fori_loop(0, n, body, 0, unroll=UNROLL if n % UNROLL == 0 else 1)

    def issue_kv(u):
        issue(kv_stream(k_hbm, k_buf, k_sems, (u + DSH) % n_steps, u % NK),
              kv_stream(v_hbm, v_buf, v_sems, u, v_slot(u)), ND, K_THREAD)

    def issue_qo(off, n):
        issue(w_stream(wq_hbm, wq_buf, w_sems.at[0], off), w_stream(wo_hbm, wo_buf, w_sems.at[1], off), n, 0)

    def issue_gu(off, n):
        issue(w_stream(wg_hbm, wg_buf, w_sems.at[2], off), w_stream(wu_hbm, wu_buf, w_sems.at[3], off), n, 0)

    wd_seq = _w_down_schedule(D)

    def issue_wd(lo, hi):
        for t, r, c, w, si in wd_seq[lo:hi]:
            pltpu.make_async_copy(wd_hbm.at[:, pl.ds(r, 8), pl.ds(c, w)], wd_buf.at[:, pl.ds(r, 8), pl.ds(c, w)],
                                  d_sems.at[si]).start(priority=t)

    def wait_all(buf, sem):
        pltpu.make_async_copy(buf, buf, sem).wait()

    def x_matmul(w_buf, store, cb=512):
        s, r, c = w_buf.shape

        def body(j, carry):
            c0 = pl.multiple_of(j * cb, 128)
            w = w_buf[:, :, pl.ds(c0, cb)].reshape(s * r, cb)
            store(j, c0, _dot(x_scr[...].astype(jnp.bfloat16), w))
            return carry
        jax.lax.fori_loop(0, c // cb, body, 0)

    small = [
        pltpu.make_async_copy(x_hbm, x_buf, w_sems.at[4]),
        pltpu.make_async_copy(wr_hbm, wr_buf, w_sems.at[5]),
        pltpu.make_async_copy(gw_hbm, gw_buf, w_sems.at[6]),
    ]

    issue_qo(0, 32)
    for cp in small:
        cp.start()
    issue_qo(32, n_qo - 32)
    issue_kv(0)

    for cp in small:
        cp.wait()
    x_scr[...] = jnp.concatenate([x_buf[...].astype(jnp.float32), jnp.zeros((M - B, D), jnp.float32)], axis=0)

    wait_all(wq_buf, w_sems.at[0])

    def store_q(j, c0, r):
        r = r.astype(jnp.bfloat16).astype(jnp.float32)
        nh = r.shape[1] // DH
        for b in range(B):
            for t in range(nh):
                q_scr[pl.ds(b * H + j * nh + t, 1), :] = r[b:b + 1, t * DH:(t + 1) * DH]
    x_matmul(wq_buf, store_q)
    acc_scr[...] = jnp.zeros_like(acc_scr)

    def prefill(u, c):
        issue_kv(u)
        return c
    jax.lax.fori_loop(1, AH, prefill, 0)
    wait_all(wo_buf, w_sems.at[1])

    scale = DH ** -0.5
    row_s = jax.lax.broadcasted_iota(jnp.int32, (M, span), 0)
    row_o = jax.lax.broadcasted_iota(jnp.int32, (M, DH), 0)
    row_d = jax.lax.broadcasted_iota(jnp.int32, (M, D), 0)
    row_g = jax.lax.broadcasted_iota(jnp.int32, (G, G * DH), 0)
    col_g = jax.lax.broadcasted_iota(jnp.int32, (G, G * DH), 1)
    segs_per_group = G * DH // wo_buf.shape[1]

    def step(t, c):
        blk = (t + DSH) % n_steps
        kslot = t % NK
        vslot = v_slot(blk)
        grp = blk // J
        jj = blk % J
        u = t + AH

        @pl.when(u < n_steps)
        def _():
            issue_kv(u)

        @pl.when(u >= n_steps)
        def _():
            issue_gu((u - n_steps) * GU_BURST, GU_BURST)

        resume = t == n_steps - DSH
        suspend = t == J - 1 - DSH

        @pl.when(jnp.logical_or(t == 0, jnp.logical_and(jj == 0, jnp.logical_not(resume))))
        def _():
            st_scr[0] = jnp.full((M, DH), -jnp.inf, jnp.float32)
            st_scr[1] = jnp.zeros((M, DH), jnp.float32)
            st_scr[2] = jnp.zeros((M, DH), jnp.float32)

        @pl.when(resume)
        def _():
            st_scr[...] = sv_scr[...]

        wait_all(k_buf.at[kslot], k_sems.at[kslot])
        q = q_scr[pl.ds(pl.multiple_of(grp * G, G), G), :].astype(jnp.bfloat16)
        s = _dot(q, k_buf[kslot, 0], _NT)
        for h in range(1, G):
            s = jnp.where(row_s == h, _dot(q, k_buf[kslot, h], _NT), s)
        s = s * scale
        m_old = st_scr[0]
        m_new = jnp.maximum(m_old, jnp.max(s, axis=-1, keepdims=True))
        alpha = jnp.exp(m_old - m_new)
        p = jnp.exp(s - m_new[:, :1])
        st_scr[1] = st_scr[1] * alpha + jnp.sum(p, axis=-1, keepdims=True)
        st_scr[0] = m_new
        pb = p.astype(jnp.bfloat16)

        wait_all(v_buf.at[vslot], v_sems.at[vslot])
        o = _dot(pb, v_buf[vslot, 0])
        for h in range(1, G):
            o = jnp.where(row_o == h, _dot(pb, v_buf[vslot, h]), o)
        st_scr[2] = st_scr[2] * alpha + o

        @pl.when(suspend)
        def _():
            sv_scr[...] = st_scr[...]

        @pl.when(jnp.logical_or(t == n_steps - 1, jnp.logical_and(jj == J - 1, jnp.logical_not(suspend))))
        def _():
            on = st_scr[2] / st_scr[1]
            obd = jnp.where(col_g // DH == row_g, jnp.concatenate([on] * G, axis=1), 0.0).astype(jnp.bfloat16)
            hg = grp % (H // G)
            w = wo_buf[pl.ds(hg * segs_per_group, segs_per_group)].reshape(G * DH, D)
            a = jnp.sum(_dot(obd, w), axis=0, keepdims=True)
            acc_scr[...] += jnp.where(row_d == grp // (H // G), a, 0.0)
        return c

    jax.lax.fori_loop(0, n_steps, step, 0)

    if n_gu > AH * GU_BURST:
        issue_gu(AH * GU_BURST, n_gu - AH * GU_BURST)
    b1, b2, b3 = BURSTS[0], BURSTS[0] + BURSTS[1], sum(BURSTS)
    issue_wd(0, b1)
    wait_all(wg_buf, w_sems.at[2])

    def store_gate(j, c0, r):
        hid_scr[:, pl.ds(c0, r.shape[1])] = r * _sigmoid(r)
    x_matmul(wg_buf, store_gate)
    issue_wd(b1, b2)
    wait_all(wu_buf, w_sems.at[3])

    def store_up(j, c0, r):
        hid_scr[:, pl.ds(c0, r.shape[1])] = hid_scr[:, pl.ds(c0, r.shape[1])] * r
    x_matmul(wu_buf, store_up)
    issue_wd(b2, b3)

    xf = x_scr[...]
    wr = wr_buf[...].astype(jnp.float32).reshape(1, D)
    gw = gw_buf[...].astype(jnp.float32).reshape(1, D)
    r_sel = _sigmoid(jnp.sum(xf * wr, axis=-1, keepdims=True))
    g = _sigmoid(jnp.sum(xf * gw, axis=-1, keepdims=True))
    base = g * acc_scr[...] + (1.0 - g) * (xf + xf * 0.0)
    coef = (1.0 - g) * r_sel

    def down(piece, c0, nc):
        r0 = piece * 128
        y = None
        for sg in range(nseg_d):
            lo = sg * SEG_D + r0
            t = _dot(hid_scr[:, lo:lo + 128].astype(jnp.bfloat16), wd_buf[sg, r0:r0 + 128, c0:c0 + nc])
            y = t if y is None else y + t
        return y

    y = None
    for p in range(3):
        wait_all(wd_buf.at[:, pl.ds(p * 128, 128), :], d_sems.at[p])
        y = down(p, 0, D) if y is None else y + down(p, 0, D)
        if p == 0:
            issue_wd(b3, len(wd_seq))
    c0 = 0
    for t, nc in enumerate(LAST_COLS):
        wait_all(wd_buf.at[:, pl.ds(384, 128), pl.ds(c0, nc)], d_sems.at[3 + t])
        yc = y[:, c0:c0 + nc] + down(3, c0, nc)
        o_ref[:, c0:c0 + nc] = (base[:, c0:c0 + nc] + coef * yc)[:B].astype(o_ref.dtype)
        c0 += nc


@jax.jit
def pallas_gated_mix__mha_block_cached__moe_arch_mod__decode_kernel(
    A_x: jax.Array,
    A_k_cache: jax.Array,
    A_v_cache: jax.Array,
    A_wq: jax.Array,
    A_wo: jax.Array,
    B_x: jax.Array,
    B_w_r: jax.Array,
    B_w_gate: jax.Array,
    B_w_up: jax.Array,
    B_w_down: jax.Array,
    gate_w: jax.Array,
):
    del B_x
    B, _, D = A_x.shape
    _, H, SK, DH = A_k_cache.shape
    F = B_w_gate.shape[1]
    bf, f32 = jnp.bfloat16, jnp.float32
    span = min(SPAN, SK // 8)
    kv_shape = (B * H // G, G, SK, DH)
    wq = A_wq.reshape(WSEG, D // WSEG, H * DH)
    wo = A_wo.reshape(WSEG, H * DH // WSEG, D)
    wg = B_w_gate.reshape(WSEG, D // WSEG, F)
    wu = B_w_up.reshape(WSEG, D // WSEG, F)
    wd = B_w_down.reshape(F // SEG_D, SEG_D, D)
    out = pl.pallas_call(
        _kernel,
        in_specs=[pl.BlockSpec(memory_space=pl.ANY)] * 10,
        out_specs=pl.BlockSpec(memory_space=pltpu.VMEM),
        out_shape=jax.ShapeDtypeStruct((B, D), A_x.dtype),
        scratch_shapes=[
            pltpu.VMEM((B, D), bf),
            pltpu.VMEM((D,), bf),
            pltpu.VMEM((D,), bf),
            pltpu.VMEM(wq.shape, bf),
            pltpu.VMEM(wo.shape, bf),
            pltpu.VMEM(wg.shape, bf),
            pltpu.VMEM(wu.shape, bf),
            pltpu.VMEM(wd.shape, bf),
            pltpu.VMEM((NV + DSH, G, span, DH), bf),
            pltpu.VMEM((NV + DSH, G, span, DH), bf),
            pltpu.VMEM((B * H, DH), f32),
            pltpu.VMEM((M, D), f32),
            pltpu.VMEM((M, F), f32),
            pltpu.VMEM((M, D), f32),
            pltpu.VMEM((3, M, DH), f32),
            pltpu.VMEM((3, M, DH), f32),
            pltpu.SemaphoreType.DMA((NV + DSH,)),
            pltpu.SemaphoreType.DMA((NV + DSH,)),
            pltpu.SemaphoreType.DMA((7,)),
            pltpu.SemaphoreType.DMA((3 + len(LAST_COLS),)),
        ],
        compiler_params=pltpu.CompilerParams(
            vmem_limit_bytes=100 * 1024 * 1024,
            disable_bounds_checks=True,
            disable_semaphore_checks=True,
        ),
    )(A_x.reshape(B, D), A_k_cache.reshape(kv_shape), A_v_cache.reshape(kv_shape),
      wq, wo, B_w_r, wg, wu, wd, gate_w)
    return out.reshape(B, 1, D)
```

```python
import functools
import jax
import jax.numpy as jnp
import jax.experimental.pallas as pl
import jax.experimental.pallas.tpu as pltpu

B, D = 4, 1024
H, SK, DH = 32, 8192, 128
F = 3584
M = 8
G = 8
NSEG_D, SEG_D = 7, 512
WC = 256

_NT = (((1,), (1,)), ((), ()))
_NN = (((1,), (0,)), ((), ()))


def _dot(a, b, dims=_NN):
    return jax.lax.dot_general(a, b, dims, preferred_element_type=jnp.float32)


def _sigmoid(x):
    return 1.0 / (1.0 + jnp.exp(-x))


def make(NS=3, HG=2, O=1, span=1024, compute=True, kth=1, skew=20, lead=0, last_cols=(768, 128, 128), bursts=(76, 62, 62), unroll=2,
         qth=0, gth=0, gu_burst=64, solo=2, pre_pairs=0, c_pro=True, c_loop=True, c_tail=True):
    weights = kvon = True
    rows = 16
    P = G // HG
    R = SK // P
    ND = span // rows
    J = R // span
    NH = B * H
    n_groups = NH // HG
    n_steps = n_groups * J
    assert skew % 2 == 0 and HG == 2 and sum(last_cols) == D and lead % 2 == 0 and 0 <= O < HG and R % span == 0
    tK = kth
    AH = NS - 1
    n_gu = D // 64 * (F // WC)
    assert AH * gu_burst <= n_gu
    wrap_grp = n_groups - 1
    SO = O * P

    def kernel(x_hbm, k_hbm, v_hbm, wq_hbm, wo_hbm, wr_hbm, wg_hbm, wu_hbm, wd_hbm, gw_hbm,
               o_ref,
               x_buf, wr_buf, gw_buf, wq_buf, wo_buf, wg_buf, wu_buf, wd_buf,
               k_buf, v_buf, q_scr, acc_scr, hid_scr, x_scr, st_scr,
               k_sems, v_sems, w_sems, d_sems):

        def mo(x, m):
            return x if isinstance(x, int) else pl.multiple_of(x, m)

        def w_stream(src, dst, sem, off=0):
            ncb = src.shape[2] // WC

            def f(j):
                j = j + off
                r = mo((j // ncb) * 8, 8)
                c = mo((j % ncb) * WC, 128)
                return pltpu.make_async_copy(src.at[:, pl.ds(r, 8), pl.ds(c, WC)],
                                             dst.at[:, pl.ds(r, 8), pl.ds(c, WC)], sem)
            return f

        def loop(n, body):
            def b(j, c):
                body(j)
                return c
            jax.lax.fori_loop(0, n, b, 0, unroll=unroll if n % unroll == 0 else 1)

        def issue(f0, f1, n):
            if n == 0:
                return

            def body(j):
                if f1 is not None:
                    f1(j).start(priority=1)
                if f0 is not None:
                    f0(j).start(priority=0)
            loop(n, body)

        kv_of = ((k_hbm, k_buf, k_sems), (v_hbm, v_buf, v_sems))
        kv_t = (kv_of[1], kv_of[0]) if kth == 1 else kv_of
        nslots_t = (NS, NS + 1)

        def kv_stream(th, u, wrap, off):
            hbm, buf, sems = kv_t[th]
            slot = u % nslots_t[th]
            base = mo((u % J) * span, span)

            def f(j):
                j = j + off
                if wrap:
                    part = j % 2
                    s0 = jnp.where(part == 0, SO + wrap_grp * G, 0) if not isinstance(part, int) else (SO + wrap_grp * G if part == 0 else 0)
                    r = mo((j // 2) * 2 * rows, 2 * rows)
                    return pltpu.make_async_copy(hbm.at[pl.ds(s0, G // 2), pl.ds(base + r, 2 * rows), :],
                                                 buf.at[slot, pl.ds(part * (G // 2), G // 2), pl.ds(r, 2 * rows), :], sems.at[slot])
                r = mo(j * rows, rows)
                return pltpu.make_async_copy(hbm.at[pl.ds(SO + (u // J) * G, G), pl.ds(base + r, rows), :],
                                             buf.at[slot, :, pl.ds(r, rows), :], sems.at[slot])
            return f

        gu_t = ((wg_hbm, wg_buf, w_sems.at[2]), (wu_hbm, wu_buf, w_sems.at[3]))
        if gth == 1:
            gu_t = gu_t[::-1]
        qo_t = ((wq_hbm, wq_buf, w_sems.at[0]), (wo_hbm, wo_buf, w_sems.at[1]))
        if qth == 1:
            qo_t = qo_t[::-1]

        def issue_kv(u):
            first_wrap = wrap_grp * J if O else 10 ** 6

            def part_a(w):
                issue(kv_stream(0, u, w, 0), kv_stream(1, u, w, skew), ND - skew)

            def part_b(w0, w1):
                nxt = w_stream(*gu_t[1]) if w1 is None else kv_stream(1, u + 1, w1, 0)
                issue(kv_stream(0, u, w0, ND - skew), nxt, skew)

            if isinstance(u, int):
                part_a(u >= first_wrap)
                part_b(u >= first_wrap, None if u == n_steps - 1 else u + 1 >= first_wrap)
                return
            if O:
                pl.when(u < first_wrap)(functools.partial(part_a, False))
                pl.when(u >= first_wrap)(functools.partial(part_a, True))
                pl.when(u < first_wrap - 1)(functools.partial(part_b, False, False))
                pl.when(u == first_wrap - 1)(functools.partial(part_b, False, True))
                if J > 1:
                    pl.when(jnp.logical_and(u >= first_wrap, u < n_steps - 1))(functools.partial(part_b, True, True))
                pl.when(u == n_steps - 1)(functools.partial(part_b, True, None))
            else:
                part_a(False)
                pl.when(u < n_steps - 1)(functools.partial(part_b, False, False))
                pl.when(u == n_steps - 1)(functools.partial(part_b, False, None))

        def issue_gu(off, n):
            issue(w_stream(*gu_t[0], off), w_stream(*gu_t[1], off + skew), n)

        def wait_all(buf, sem):
            pltpu.make_async_copy(buf, buf, sem).wait()

        wait_w = wait_all

        small = [
            pltpu.make_async_copy(x_hbm, x_buf, w_sems.at[4]),
            pltpu.make_async_copy(wr_hbm, wr_buf, w_sems.at[5]),
            pltpu.make_async_copy(gw_hbm, gw_buf, w_sems.at[6]),
        ]

        batches = [(0, 0, 0, D), (1, 128, 0, D), (2, 256, 0, D)]
        c0 = 0
        for t, nc in enumerate(last_cols):
            batches.append((3 + t, 384, c0, nc))
            c0 += nc
        L = [[], []]
        for bi, (si, r0, c0, nc) in enumerate(batches):
            w = min(WC, nc)
            assert nc % w == 0
            ds = [(r, c, w, si) for r in range(r0, r0 + 128, 8) for c in range(c0, c0 + nc, w)]
            n0 = len(ds) // 2 + (lead // 2 if bi == 0 else 0)
            if bi >= len(batches) - solo:
                n0 = 0
            L[0] += ds[:n0]
            L[1] += ds[n0:]
        seq = []
        for j in range(0, max(len(L[0]), len(L[1]))):
            if j + skew < len(L[1]):
                seq.append((1, L[1][j + skew]))
            if j < len(L[0]):
                seq.append((0, L[0][j]))
        n0_p0 = 32 + lead // 2
        assert skew <= 64 - n0_p0

        def issue_seq(lo, hi):
            for t, item in seq[lo:hi]:
                if isinstance(item, int):
                    w_stream(*gu_t[0])(item).start(priority=0)
                    continue
                r, c, w, si = item
                pltpu.make_async_copy(wd_hbm.at[:, pl.ds(r, 8), pl.ds(c, w)], wd_buf.at[:, pl.ds(r, 8), pl.ds(c, w)],
                                      d_sems.at[si]).start(priority=t)

        if pre_pairs:
            issue(w_stream(*qo_t[0]), w_stream(*qo_t[1]), pre_pairs)
        issue(None, w_stream(*qo_t[1], pre_pairs), skew)
        for c in small:
            c.start()
        issue(w_stream(*qo_t[0], pre_pairs), w_stream(*qo_t[1], pre_pairs + skew), 256 - skew - pre_pairs)
        issue(w_stream(*qo_t[0], 256 - skew), kv_stream(1, 0, False, 0), skew)
        issue_kv(0)

        for c in small:
            c.wait()
        x_scr[...] = jnp.concatenate([x_buf[...].astype(jnp.float32), jnp.zeros((M - B, D), jnp.float32)], axis=0)

        def colmm(w_buf, cb, store):
            S, R_, C = w_buf.shape

            def body(j, c):
                c0 = pl.multiple_of(j * cb, 128)
                w = w_buf[:, :, pl.ds(c0, cb)].reshape(S * R_, cb)
                store(j, c0, _dot(x_scr[...].astype(jnp.bfloat16), w))
                return c
            jax.lax.fori_loop(0, C // cb, body, 0)

        wait_w(wq_buf, w_sems.at[0])
        if compute and c_pro:
            def st_q(j, c0, r):
                r = r.astype(jnp.bfloat16).astype(jnp.float32)
                for b in range(B):
                    for t in range(4):
                        q_scr[pl.ds(b * H + j * 4 + t, 1), :] = r[b:b + 1, t * DH:(t + 1) * DH]
            colmm(wq_buf, 512, st_q)
        acc_scr[...] = jnp.zeros_like(acc_scr)

        for u in range(1, AH):
            issue_kv(u)
        wait_w(wo_buf, w_sems.at[1])

        scale = DH ** -0.5
        row_s = jax.lax.broadcasted_iota(jnp.int32, (M, span), 0)
        row_o = jax.lax.broadcasted_iota(jnp.int32, (M, DH), 0)
        head_o = row_o // P

        def step_body(t, c):
            kslot = t % nslots_t[tK]
            vslot = t % nslots_t[1 - tK]
            grp = t // J
            jj = t % J
            u = t + AH

            @pl.when(u < n_steps)
            def _():
                issue_kv(u)

            @pl.when(u >= n_steps)
            def _():
                issue_gu((u - n_steps) * gu_burst, gu_burst)

            @pl.when(jj == 0)
            def _():
                st_scr[0] = jnp.full((M, DH), -jnp.inf, jnp.float32)
                st_scr[1] = jnp.zeros((M, DH), jnp.float32)
                st_scr[2] = jnp.zeros((M, DH), jnp.float32)

            heads = [(grp * HG + O + a) % NH for a in range(HG)]
            if kvon:
                wait_all(k_buf.at[kslot], k_sems.at[kslot])
            if compute and c_loop:
                q = jnp.broadcast_to(q_scr[pl.ds(heads[0], 1), :], (M, DH))
                for a in range(1, HG):
                    q = jnp.where(head_o == a, q_scr[pl.ds(heads[a], 1), :], q)
                q = q.astype(jnp.bfloat16)
                s = _dot(q, k_buf[kslot, 0], _NT)
                for h in range(1, G):
                    s = jnp.where(row_s == h, _dot(q, k_buf[kslot, h], _NT), s)
                s = s * scale
                m_old = st_scr[0]
                m_new = jnp.maximum(m_old, jnp.max(s, axis=-1, keepdims=True))
                alpha = jnp.exp(m_old - m_new)
                p = jnp.exp(s - m_new[:, :1])
                st_scr[1] = st_scr[1] * alpha + jnp.sum(p, axis=-1, keepdims=True)
                st_scr[0] = m_new
                pb = p.astype(jnp.bfloat16)
            if kvon:
                wait_all(v_buf.at[vslot], v_sems.at[vslot])
            if compute and c_loop:
                o = _dot(pb, v_buf[vslot, 0])
                for h in range(1, G):
                    o = jnp.where(row_o == h, _dot(pb, v_buf[vslot, h]), o)
                st_scr[2] = st_scr[2] * alpha + o

                @pl.when(jj == J - 1)
                def _():
                    m, l, o = st_scr[0], st_scr[1], st_scr[2]
                    acc = acc_scr[...]
                    for a in range(HG):
                        mine = head_o == a
                        mh = jnp.max(jnp.where(mine, m, -jnp.inf), axis=0, keepdims=True)
                        w = jnp.where(mine, jnp.exp(m - mh), 0.0)
                        lh = jnp.sum(w * l, axis=0, keepdims=True)
                        oh = jnp.sum(w * o, axis=0, keepdims=True) / lh
                        h = heads[a] % H
                        lhs = jnp.where(row_o == heads[a] // H, oh, 0.0).astype(jnp.bfloat16)
                        acc = acc + _dot(lhs, wo_buf[h // 4, pl.ds(pl.multiple_of((h % 4) * DH, DH), DH), :])
                    acc_scr[...] = acc
            return c

        jax.lax.fori_loop(0, n_steps, step_body, 0)

        ct = compute and c_tail
        done = AH * gu_burst
        assert n_gu - skew >= done
        issue_gu(done, n_gu - skew - done)
        issue(w_stream(*gu_t[0], n_gu - skew), w_stream(wd_hbm, wd_buf, d_sems.at[0], n0_p0), skew)
        b1, b2, b3 = bursts[0], bursts[0] + bursts[1], sum(bursts)
        issue_seq(0, b1)
        wait_w(wg_buf, w_sems.at[2])
        if ct:
            def st_g(j, c0, r):
                hid_scr[:, pl.ds(c0, 512)] = r * _sigmoid(r)
            colmm(wg_buf, 512, st_g)
        issue_seq(b1, b2)
        wait_w(wu_buf, w_sems.at[3])
        if ct:
            def st_u(j, c0, r):
                hid_scr[:, pl.ds(c0, 512)] = hid_scr[:, pl.ds(c0, 512)] * r
            colmm(wu_buf, 512, st_u)
        issue_seq(b2, b3)

        xf = x_scr[...]
        wr = wr_buf[...].astype(jnp.float32).reshape(1, D)
        gw = gw_buf[...].astype(jnp.float32).reshape(1, D)
        r_sel = _sigmoid(jnp.sum(xf * wr, axis=-1, keepdims=True))
        g = _sigmoid(jnp.sum(xf * gw, axis=-1, keepdims=True))
        base = g * acc_scr[...] + (1.0 - g) * (xf + xf * 0.0)
        coef = (1.0 - g) * r_sel

        def down(piece, c0, nc):
            r0 = piece * 128
            y = None
            for sg in range(NSEG_D):
                lo = sg * SEG_D + r0
                t = _dot(hid_scr[:, lo:lo + 128].astype(jnp.bfloat16), wd_buf[sg, r0:r0 + 128, c0:c0 + nc])
                y = t if y is None else y + t
            return y

        y = jnp.zeros((M, D), jnp.float32)
        for p in range(3):
            wait_w(wd_buf.at[:, pl.ds(p * 128, 128), :], d_sems.at[p])
            if ct:
                y = y + down(p, 0, D)
            if p == 0:
                issue_seq(b3, len(seq))
        c0 = 0
        for t, nc in enumerate(last_cols):
            wait_w(wd_buf.at[:, pl.ds(384, 128), pl.ds(c0, nc)], d_sems.at[3 + t])
            yc = y[:, c0:c0 + nc]
            if ct:
                yc = yc + down(3, c0, nc)
            o_ref[:, c0:c0 + nc] = (base[:, c0:c0 + nc] + coef * yc)[:B].astype(o_ref.dtype)
            c0 += nc

    @jax.jit
    def fn(A_x, A_k_cache, A_v_cache, A_wq, A_wo, B_x, B_w_r, B_w_gate, B_w_up, B_w_down, gate_w):
        bf = jnp.bfloat16
        wq = A_wq.reshape(8, D // 8, H * DH)
        wg = B_w_gate.reshape(8, D // 8, F)
        wu = B_w_up.reshape(8, D // 8, F)
        wo = A_wo.reshape(8, 512, D)
        wd = B_w_down.reshape(NSEG_D, SEG_D, D)
        kv_shape = (NH * P, R, DH)
        out = pl.pallas_call(
            kernel,
            in_specs=[pl.BlockSpec(memory_space=pl.ANY)] * 10,
            out_specs=pl.BlockSpec(memory_space=pltpu.VMEM),
            out_shape=jax.ShapeDtypeStruct((B, D), A_x.dtype),
            scratch_shapes=[
                pltpu.VMEM((B, D), bf),
                pltpu.VMEM((D,), bf),
                pltpu.VMEM((D,), bf),
                pltpu.VMEM(wq.shape, bf),
                pltpu.VMEM(wo.shape, bf),
                pltpu.VMEM(wg.shape, bf),
                pltpu.VMEM(wu.shape, bf),
                pltpu.VMEM(wd.shape, bf),
                pltpu.VMEM((NS + tK, G, span, DH), bf),
                pltpu.VMEM((NS + 1 - tK, G, span, DH), bf),
                pltpu.VMEM((NH, DH), jnp.float32),
                pltpu.VMEM((M, D), jnp.float32),
                pltpu.VMEM((M, F), jnp.float32),
                pltpu.VMEM((M, D), jnp.float32),
                pltpu.VMEM((3, M, DH), jnp.float32),
                pltpu.SemaphoreType.DMA((NS + tK,)),
                pltpu.SemaphoreType.DMA((NS + 1 - tK,)),
                pltpu.SemaphoreType.DMA((7,)),
                pltpu.SemaphoreType.DMA((3 + len(last_cols),)),
            ],
            compiler_params=pltpu.CompilerParams(
                vmem_limit_bytes=100 * 1024 * 1024,
                disable_bounds_checks=True,
                disable_semaphore_checks=True,
            ),
        )(A_x.reshape(B, D), A_k_cache.reshape(kv_shape), A_v_cache.reshape(kv_shape),
          wq, wo, B_w_r, wg, wu, wd, gate_w)
        return out.reshape(B, 1, D)
    return fn


_IMPL = make(skew=16, kth=0)


@jax.jit
def pallas_gated_mix__mha_block_cached__moe_arch_mod__decode_kernel(
    A_x: jax.Array,
    A_k_cache: jax.Array,
    A_v_cache: jax.Array,
    A_wq: jax.Array,
    A_wo: jax.Array,
    B_x: jax.Array,
    B_w_r: jax.Array,
    B_w_gate: jax.Array,
    B_w_up: jax.Array,
    B_w_down: jax.Array,
    gate_w: jax.Array,
):
    return _IMPL(A_x, A_k_cache, A_v_cache, A_wq, A_wo, B_x, B_w_r, B_w_gate, B_w_up, B_w_down, gate_w)
```

```python
import functools

import jax
import jax.numpy as jnp
import jax.experimental.pallas as pl
import jax.experimental.pallas.tpu as pltpu

M = 8
G = 8
HG = 2
P = G // HG
HEAD0 = 1
ROWS = 16
SPAN = 1024
NS = 3
SKEW = 24
WSEG = 8
WC = 256
SEG_D = 512
GU_BURST = 64
LAST_COLS = (768, 128, 128)
SOLO = 2
BURSTS = (76, 62, 62)

_NT = (((1,), (1,)), ((), ()))
_NN = (((1,), (0,)), ((), ()))


def _dot(a, b, dims=_NN):
    return jax.lax.dot_general(a, b, dims, preferred_element_type=jnp.float32)


def _sigmoid(x):
    return 1.0 / (1.0 + jnp.exp(-x))


def _mo(x, m):
    return x if isinstance(x, int) else pl.multiple_of(x, m)


def _w_down_schedule(d, skew):
    batches = [(p, p * 128, 0, d) for p in range(3)]
    c0 = 0
    for t, nc in enumerate(LAST_COLS):
        batches.append((3 + t, 384, c0, nc))
        c0 += nc
    assert c0 == d
    lists = [[], []]
    for bi, (si, r0, c0, nc) in enumerate(batches):
        w = min(WC, nc)
        assert nc % w == 0
        ds = [(r, c, w, si) for r in range(r0, r0 + 128, 8) for c in range(c0, c0 + nc, w)]
        n0 = 0 if bi >= len(batches) - SOLO else len(ds) // 2
        lists[0] += ds[:n0]
        lists[1] += ds[n0:]
    seq = []
    for j in range(max(len(lists[0]), len(lists[1]))):
        if j + skew < len(lists[1]):
            seq.append((1,) + lists[1][j + skew])
        if j < len(lists[0]):
            seq.append((0,) + lists[0][j])
    return seq


def _kernel(x_hbm, k_hbm, v_hbm, wq_hbm, wo_hbm, wr_hbm, wg_hbm, wu_hbm, wd_hbm, gw_hbm,
            o_ref,
            x_buf, wr_buf, gw_buf, wq_buf, wo_buf, wg_buf, wu_buf, wd_buf,
            k_buf, v_buf, q_scr, acc_scr, hid_scr, x_scr, st_scr,
            k_sems, v_sems, w_sems, d_sems):
    B, D = x_buf.shape
    n_seg, R, DH = k_hbm.shape
    NH = n_seg // P
    H = NH // B
    span = k_buf.shape[2]
    nseg_d = wd_buf.shape[0]
    AH = NS - 1
    ND = span // ROWS
    J = R // span
    n_groups = NH // HG
    n_steps = n_groups * J
    first_wrap = (n_groups - 1) * J
    seg0 = HEAD0 * P
    skew = min(SKEW, ND // 2)
    n_qo = wq_buf.shape[1] // 8 * (wq_buf.shape[2] // WC)
    n_gu = wg_buf.shape[1] // 8 * (wg_buf.shape[2] // WC)
    n_p0 = 128 // 8 * (D // WC)
    assert n_qo == wo_buf.shape[1] // 8 * (wo_buf.shape[2] // WC)
    assert seg0 == G // 2 and skew % 2 == 0 and ND % 2 == 0 and skew <= n_p0 // 2 and AH < first_wrap
    assert AH * GU_BURST + skew <= n_gu and wd_buf.shape[1] == SEG_D == 512

    def kv_stream(thread, u, wrap, off):
        hbm, buf, sems = ((k_hbm, k_buf, k_sems), (v_hbm, v_buf, v_sems))[thread]
        slot = u % (NS + thread)
        base = _mo((u % J) * span, span)

        def f(j):
            j = j + off
            if wrap:
                half = j % 2
                r = _mo((j // 2) * 2 * ROWS, 2 * ROWS)
                src = (1 - half) * (n_seg - P)
                return pltpu.make_async_copy(hbm.at[pl.ds(src, P), pl.ds(base + r, 2 * ROWS), :],
                                             buf.at[slot, pl.ds(half * P, P), pl.ds(r, 2 * ROWS), :], sems.at[slot])
            r = _mo(j * ROWS, ROWS)
            return pltpu.make_async_copy(hbm.at[pl.ds(seg0 + (u // J) * G, G), pl.ds(base + r, ROWS), :],
                                         buf.at[slot, :, pl.ds(r, ROWS), :], sems.at[slot])
        return f

    def w_stream(src, dst, sem, off):
        ncb = src.shape[2] // WC

        def f(j):
            j = j + off
            r = _mo((j // ncb) * 8, 8)
            c = _mo((j % ncb) * WC, 128)
            return pltpu.make_async_copy(src.at[:, pl.ds(r, 8), pl.ds(c, WC)],
                                         dst.at[:, pl.ds(r, 8), pl.ds(c, WC)], sem)
        return f

    wq_stream = functools.partial(w_stream, wq_hbm, wq_buf, w_sems.at[0])
    wo_stream = functools.partial(w_stream, wo_hbm, wo_buf, w_sems.at[1])
    wg_stream = functools.partial(w_stream, wg_hbm, wg_buf, w_sems.at[2])
    wu_stream = functools.partial(w_stream, wu_hbm, wu_buf, w_sems.at[3])

    def issue(f0, f1, n):
        def body(j, c):
            f1(j).start(priority=1)
            if f0 is not None:
                f0(j).start(priority=0)
            return c
        jax.lax.fori_loop(0, n, body, 0)

    def issue_kv(u):
        def part_a(wrap):
            issue(kv_stream(0, u, wrap, 0), kv_stream(1, u, wrap, skew), ND - skew)

        def part_b(wrap, next_wrap):
            nxt = wu_stream(0) if next_wrap is None else kv_stream(1, u + 1, next_wrap, 0)
            issue(kv_stream(0, u, wrap, ND - skew), nxt, skew)

        if isinstance(u, int):
            part_a(False)
            part_b(False, False)
            return
        pl.when(u < first_wrap)(functools.partial(part_a, False))
        pl.when(u >= first_wrap)(functools.partial(part_a, True))
        pl.when(u < first_wrap - 1)(functools.partial(part_b, False, False))
        pl.when(u == first_wrap - 1)(functools.partial(part_b, False, True))
        if J > 1:
            pl.when(jnp.logical_and(u >= first_wrap, u < n_steps - 1))(functools.partial(part_b, True, True))
        pl.when(u == n_steps - 1)(functools.partial(part_b, True, None))

    def issue_gu(off, n):
        issue(wg_stream(off), wu_stream(off + skew), n)

    wd_seq = _w_down_schedule(D, skew)

    def issue_wd(lo, hi):
        for t, r, c, w, si in wd_seq[lo:hi]:
            pltpu.make_async_copy(wd_hbm.at[:, pl.ds(r, 8), pl.ds(c, w)], wd_buf.at[:, pl.ds(r, 8), pl.ds(c, w)],
                                  d_sems.at[si]).start(priority=t)

    def wait_all(buf, sem):
        pltpu.make_async_copy(buf, buf, sem).wait()

    def x_matmul(w_buf, store, cb=512):
        s, r, c = w_buf.shape

        def body(j, carry):
            c0 = pl.multiple_of(j * cb, 128)
            w = w_buf[:, :, pl.ds(c0, cb)].reshape(s * r, cb)
            store(j, c0, _dot(x_scr[...].astype(jnp.bfloat16), w))
            return carry
        jax.lax.fori_loop(0, c // cb, body, 0)

    small = [
        pltpu.make_async_copy(x_hbm, x_buf, w_sems.at[4]),
        pltpu.make_async_copy(wr_hbm, wr_buf, w_sems.at[5]),
        pltpu.make_async_copy(gw_hbm, gw_buf, w_sems.at[6]),
    ]

    issue(None, wo_stream(0), skew)
    for cp in small:
        cp.start()
    issue(wq_stream(0), wo_stream(skew), n_qo - skew)
    issue(wq_stream(n_qo - skew), kv_stream(1, 0, False, 0), skew)
    issue_kv(0)

    for cp in small:
        cp.wait()
    x_scr[...] = jnp.concatenate([x_buf[...].astype(jnp.float32), jnp.zeros((M - B, D), jnp.float32)], axis=0)

    wait_all(wq_buf, w_sems.at[0])

    def store_q(j, c0, r):
        r = r.astype(jnp.bfloat16).astype(jnp.float32)
        nh = r.shape[1] // DH
        for b in range(B):
            for t in range(nh):
                q_scr[pl.ds(b * H + j * nh + t, 1), :] = r[b:b + 1, t * DH:(t + 1) * DH]
    x_matmul(wq_buf, store_q)
    acc_scr[...] = jnp.zeros_like(acc_scr)

    for u in range(1, AH):
        issue_kv(u)
    wait_all(wo_buf, w_sems.at[1])

    scale = DH ** -0.5
    row_s = jax.lax.broadcasted_iota(jnp.int32, (M, span), 0)
    row_o = jax.lax.broadcasted_iota(jnp.int32, (M, DH), 0)
    head_o = row_o // P
    heads_per_seg = wo_buf.shape[1] // DH

    def step(t, c):
        kslot = t % NS
        vslot = t % (NS + 1)
        jj = t % J
        u = t + AH

        @pl.when(u < n_steps)
        def _():
            issue_kv(u)

        @pl.when(u >= n_steps)
        def _():
            issue_gu((u - n_steps) * GU_BURST, GU_BURST)

        @pl.when(jj == 0)
        def _():
            st_scr[0] = jnp.full((M, DH), -jnp.inf, jnp.float32)
            st_scr[1] = jnp.zeros((M, DH), jnp.float32)
            st_scr[2] = jnp.zeros((M, DH), jnp.float32)

        heads = [((t // J) * HG + HEAD0 + a) % NH for a in range(HG)]
        wait_all(k_buf.at[kslot], k_sems.at[kslot])
        q = jnp.broadcast_to(q_scr[pl.ds(heads[0], 1), :], (M, DH))
        for a in range(1, HG):
            q = jnp.where(head_o == a, q_scr[pl.ds(heads[a], 1), :], q)
        q = q.astype(jnp.bfloat16)
        s = _dot(q, k_buf[kslot, 0], _NT)
        for r in range(1, G):
            s = jnp.where(row_s == r, _dot(q, k_buf[kslot, r], _NT), s)
        s = s * scale
        m_old = st_scr[0]
        m_new = jnp.maximum(m_old, jnp.max(s, axis=-1, keepdims=True))
        alpha = jnp.exp(m_old - m_new)
        p = jnp.exp(s - m_new[:, :1])
        st_scr[1] = st_scr[1] * alpha + jnp.sum(p, axis=-1, keepdims=True)
        st_scr[0] = m_new
        pb = p.astype(jnp.bfloat16)

        wait_all(v_buf.at[vslot], v_sems.at[vslot])
        o = _dot(pb, v_buf[vslot, 0])
        for r in range(1, G):
            o = jnp.where(row_o == r, _dot(pb, v_buf[vslot, r]), o)
        st_scr[2] = st_scr[2] * alpha + o

        @pl.when(jj == J - 1)
        def _():
            m, l, o_part = st_scr[0], st_scr[1], st_scr[2]
            acc = acc_scr[...]
            for a in range(HG):
                mine = head_o == a
                m_h = jnp.max(jnp.where(mine, m, -jnp.inf), axis=0, keepdims=True)
                w = jnp.exp(m - m_h)
                l_h = jnp.sum(jnp.where(mine, w * l, 0.0), axis=0, keepdims=True)
                o_h = jnp.sum(jnp.where(mine, w * o_part, 0.0), axis=0, keepdims=True) / l_h
                h = heads[a] % H
                lhs = jnp.where(row_o == heads[a] // H, o_h, 0.0).astype(jnp.bfloat16)
                wo_h = wo_buf[h // heads_per_seg, pl.ds(pl.multiple_of((h % heads_per_seg) * DH, DH), DH), :]
                acc = acc + _dot(lhs, wo_h)
            acc_scr[...] = acc
        return c

    jax.lax.fori_loop(0, n_steps, step, 0)

    issue_gu(AH * GU_BURST, n_gu - skew - AH * GU_BURST)
    issue(wg_stream(n_gu - skew), w_stream(wd_hbm, wd_buf, d_sems.at[0], n_p0 // 2), skew)
    b1, b2, b3 = BURSTS[0], BURSTS[0] + BURSTS[1], sum(BURSTS)
    issue_wd(0, b1)
    wait_all(wg_buf, w_sems.at[2])

    def store_gate(j, c0, r):
        hid_scr[:, pl.ds(c0, r.shape[1])] = r * _sigmoid(r)
    x_matmul(wg_buf, store_gate)
    issue_wd(b1, b2)
    wait_all(wu_buf, w_sems.at[3])

    def store_up(j, c0, r):
        hid_scr[:, pl.ds(c0, r.shape[1])] = hid_scr[:, pl.ds(c0, r.shape[1])] * r
    x_matmul(wu_buf, store_up)
    issue_wd(b2, b3)

    xf = x_scr[...]
    wr = wr_buf[...].astype(jnp.float32).reshape(1, D)
    gw = gw_buf[...].astype(jnp.float32).reshape(1, D)
    r_sel = _sigmoid(jnp.sum(xf * wr, axis=-1, keepdims=True))
    g = _sigmoid(jnp.sum(xf * gw, axis=-1, keepdims=True))
    base = g * acc_scr[...] + (1.0 - g) * (xf + xf * 0.0)
    coef = (1.0 - g) * r_sel

    def down(piece, c0, nc):
        r0 = piece * 128
        y = None
        for sg in range(nseg_d):
            lo = sg * SEG_D + r0
            t = _dot(hid_scr[:, lo:lo + 128].astype(jnp.bfloat16), wd_buf[sg, r0:r0 + 128, c0:c0 + nc])
            y = t if y is None else y + t
        return y

    y = None
    for p in range(3):
        wait_all(wd_buf.at[:, pl.ds(p * 128, 128), :], d_sems.at[p])
        y = down(p, 0, D) if y is None else y + down(p, 0, D)
        if p == 0:
            issue_wd(b3, len(wd_seq))
    c0 = 0
    for t, nc in enumerate(LAST_COLS):
        wait_all(wd_buf.at[:, pl.ds(384, 128), pl.ds(c0, nc)], d_sems.at[3 + t])
        yc = y[:, c0:c0 + nc] + down(3, c0, nc)
        o_ref[:, c0:c0 + nc] = (base[:, c0:c0 + nc] + coef * yc)[:B].astype(o_ref.dtype)
        c0 += nc


@jax.jit
def pallas_gated_mix__mha_block_cached__moe_arch_mod__decode_kernel(
    A_x: jax.Array,
    A_k_cache: jax.Array,
    A_v_cache: jax.Array,
    A_wq: jax.Array,
    A_wo: jax.Array,
    B_x: jax.Array,
    B_w_r: jax.Array,
    B_w_gate: jax.Array,
    B_w_up: jax.Array,
    B_w_down: jax.Array,
    gate_w: jax.Array,
):
    del B_x
    B, _, D = A_x.shape
    _, H, SK, DH = A_k_cache.shape
    F = B_w_gate.shape[1]
    bf, f32 = jnp.bfloat16, jnp.float32
    span = min(SPAN, SK // P // 2)
    kv_shape = (B * H * P, SK // P, DH)
    wq = A_wq.reshape(WSEG, D // WSEG, H * DH)
    wo = A_wo.reshape(WSEG, H * DH // WSEG, D)
    wg = B_w_gate.reshape(WSEG, D // WSEG, F)
    wu = B_w_up.reshape(WSEG, D // WSEG, F)
    wd = B_w_down.reshape(F // SEG_D, SEG_D, D)
    out = pl.pallas_call(
        _kernel,
        in_specs=[pl.BlockSpec(memory_space=pl.ANY)] * 10,
        out_specs=pl.BlockSpec(memory_space=pltpu.VMEM),
        out_shape=jax.ShapeDtypeStruct((B, D), A_x.dtype),
        scratch_shapes=[
            pltpu.VMEM((B, D), bf),
            pltpu.VMEM((D,), bf),
            pltpu.VMEM((D,), bf),
            pltpu.VMEM(wq.shape, bf),
            pltpu.VMEM(wo.shape, bf),
            pltpu.VMEM(wg.shape, bf),
            pltpu.VMEM(wu.shape, bf),
            pltpu.VMEM(wd.shape, bf),
            pltpu.VMEM((NS, G, span, DH), bf),
            pltpu.VMEM((NS + 1, G, span, DH), bf),
            pltpu.VMEM((B * H, DH), f32),
            pltpu.VMEM((M, D), f32),
            pltpu.VMEM((M, F), f32),
            pltpu.VMEM((M, D), f32),
            pltpu.VMEM((3, M, DH), f32),
            pltpu.SemaphoreType.DMA((NS,)),
            pltpu.SemaphoreType.DMA((NS + 1,)),
            pltpu.SemaphoreType.DMA((7,)),
            pltpu.SemaphoreType.DMA((3 + len(LAST_COLS),)),
        ],
        compiler_params=pltpu.CompilerParams(
            vmem_limit_bytes=100 * 1024 * 1024,
            disable_bounds_checks=True,
            disable_semaphore_checks=True,
        ),
    )(A_x.reshape(B, D), A_k_cache.reshape(kv_shape), A_v_cache.reshape(kv_shape),
      wq, wo, B_w_r, wg, wu, wd, gate_w)
    return out.reshape(B, 1, D)
```

```python
import functools

import jax
import jax.numpy as jnp
import jax.experimental.pallas as pl
import jax.experimental.pallas.tpu as pltpu

M = 8
G = 8
HG = 2
P = G // HG
HEAD0 = 1
ROWS = 16
SPAN = 1024
NS = 3
SKEW = 24
WSEG = 8
WC = 256
SEG_D = 512
GU_BURST = 64
LAST_COLS = (768, 128, 128)
SOLO = 2
BURSTS = (76, 62, 62)

_NT = (((1,), (1,)), ((), ()))
_NN = (((1,), (0,)), ((), ()))


def _dot(a, b, dims=_NN):
    return jax.lax.dot_general(a, b, dims, preferred_element_type=jnp.float32)


def _sigmoid(x):
    return 1.0 / (1.0 + jnp.exp(-x))


def _mo(x, m):
    return x if isinstance(x, int) else pl.multiple_of(x, m)


def _w_down_schedule(d, skew):
    batches = [(p, p * 128, 0, d) for p in range(3)]
    c0 = 0
    for t, nc in enumerate(LAST_COLS):
        batches.append((3 + t, 384, c0, nc))
        c0 += nc
    assert c0 == d
    lists = [[], []]
    for bi, (si, r0, c0, nc) in enumerate(batches):
        w = min(WC, nc)
        assert nc % w == 0
        ds = [(r, c, w, si) for r in range(r0, r0 + 128, 8) for c in range(c0, c0 + nc, w)]
        n0 = 0 if bi >= len(batches) - SOLO else len(ds) // 2
        lists[0] += ds[:n0]
        lists[1] += ds[n0:]
    seq = []
    for j in range(max(len(lists[0]), len(lists[1]))):
        if j + skew < len(lists[1]):
            seq.append((1,) + lists[1][j + skew])
        if j < len(lists[0]):
            seq.append((0,) + lists[0][j])
    return seq


def _kernel(x_hbm, k_hbm, v_hbm, wq_hbm, wo_hbm, wr_hbm, wg_hbm, wu_hbm, wd_hbm, gw_hbm,
            o_ref,
            x_buf, wr_buf, gw_buf, wq_buf, wo_buf, wg_buf, wu_buf, wd_buf,
            k_buf, v_buf, q_scr, acc_scr, hid_scr, x_scr, st_scr,
            k_sems, v_sems, w_sems, d_sems):
    B, D = x_buf.shape
    n_seg, R, DH = k_hbm.shape
    NH = n_seg // P
    H = NH // B
    span = k_buf.shape[2]
    nseg_d = wd_buf.shape[0]
    AH = NS - 1
    ND = span // ROWS
    J = R // span
    n_groups = NH // HG
    n_steps = n_groups * J
    first_wrap = (n_groups - 1) * J
    seg0 = HEAD0 * P
    skew = min(SKEW, ND // 2)
    n_qo = wq_buf.shape[1] // 8 * (wq_buf.shape[2] // WC)
    n_gu = wg_buf.shape[1] // 8 * (wg_buf.shape[2] // WC)
    n_p0 = 128 // 8 * (D // WC)
    assert n_qo == wo_buf.shape[1] // 8 * (wo_buf.shape[2] // WC)
    assert seg0 == G // 2 and skew % 2 == 0 and ND % 2 == 0 and skew <= n_p0 // 2 and 2 <= AH < first_wrap
    assert AH * GU_BURST + skew <= n_gu and wd_buf.shape[1] == SEG_D == 512

    def kv_stream(thread, u, wrap, off):
        hbm, buf, sems = ((k_hbm, k_buf, k_sems), (v_hbm, v_buf, v_sems))[thread]
        slot = u % (NS + thread)
        base = _mo((u % J) * span, span)

        def f(j):
            j = j + off
            if wrap:
                half = j % 2
                r = _mo((j // 2) * 2 * ROWS, 2 * ROWS)
                src = (1 - half) * (n_seg - P)
                return pltpu.make_async_copy(hbm.at[pl.ds(src, P), pl.ds(base + r, 2 * ROWS), :],
                                             buf.at[slot, pl.ds(half * P, P), pl.ds(r, 2 * ROWS), :], sems.at[slot])
            r = _mo(j * ROWS, ROWS)
            return pltpu.make_async_copy(hbm.at[pl.ds(seg0 + (u // J) * G, G), pl.ds(base + r, ROWS), :],
                                         buf.at[slot, :, pl.ds(r, ROWS), :], sems.at[slot])
        return f

    def w_stream(src, dst, sem, off):
        ncb = src.shape[2] // WC

        def f(j):
            j = j + off
            r = _mo((j // ncb) * 8, 8)
            c = _mo((j % ncb) * WC, 128)
            return pltpu.make_async_copy(src.at[:, pl.ds(r, 8), pl.ds(c, WC)],
                                         dst.at[:, pl.ds(r, 8), pl.ds(c, WC)], sem)
        return f

    wq_stream = functools.partial(w_stream, wq_hbm, wq_buf, w_sems.at[0])
    wo_stream = functools.partial(w_stream, wo_hbm, wo_buf, w_sems.at[1])
    wg_stream = functools.partial(w_stream, wg_hbm, wg_buf, w_sems.at[2])
    wu_stream = functools.partial(w_stream, wu_hbm, wu_buf, w_sems.at[3])

    def issue(f0, f1, n):
        def body(j, c):
            f1(j).start(priority=1)
            if f0 is not None:
                f0(j).start(priority=0)
            return c
        jax.lax.fori_loop(0, n, body, 0)

    def issue_kv(u):
        def part_a(wrap):
            issue(kv_stream(0, u, wrap, 0), kv_stream(1, u, wrap, skew), ND - skew)

        def part_b(wrap, next_wrap):
            nxt = wu_stream(0) if next_wrap is None else kv_stream(1, u + 1, next_wrap, 0)
            issue(kv_stream(0, u, wrap, ND - skew), nxt, skew)

        if isinstance(u, int):
            part_a(False)
            part_b(False, False)
            return
        pl.when(u < first_wrap)(functools.partial(part_a, False))
        pl.when(u >= first_wrap)(functools.partial(part_a, True))
        pl.when(u < first_wrap - 1)(functools.partial(part_b, False, False))
        pl.when(u == first_wrap - 1)(functools.partial(part_b, False, True))
        if J > 1:
            pl.when(jnp.logical_and(u >= first_wrap, u < n_steps - 1))(functools.partial(part_b, True, True))
        pl.when(u == n_steps - 1)(functools.partial(part_b, True, None))

    def issue_gu(off, n):
        issue(wg_stream(off), wu_stream(off + skew), n)

    wd_seq = _w_down_schedule(D, skew)

    def issue_wd(lo, hi):
        for t, r, c, w, si in wd_seq[lo:hi]:
            pltpu.make_async_copy(wd_hbm.at[:, pl.ds(r, 8), pl.ds(c, w)], wd_buf.at[:, pl.ds(r, 8), pl.ds(c, w)],
                                  d_sems.at[si]).start(priority=t)

    def wait_all(buf, sem):
        pltpu.make_async_copy(buf, buf, sem).wait()

    def x_matmul(w_buf, store, cb=512, halfway=None):
        s, r, c = w_buf.shape

        def body(j, carry):
            if halfway is not None:
                pl.when(j == c // cb // 2)(halfway)
            c0 = pl.multiple_of(j * cb, 128)
            w = w_buf[:, :, pl.ds(c0, cb)].reshape(s * r, cb)
            store(j, c0, _dot(x_scr[...].astype(jnp.bfloat16), w))
            return carry
        jax.lax.fori_loop(0, c // cb, body, 0)

    small = [
        pltpu.make_async_copy(x_hbm, x_buf, w_sems.at[4]),
        pltpu.make_async_copy(wr_hbm, wr_buf, w_sems.at[5]),
        pltpu.make_async_copy(gw_hbm, gw_buf, w_sems.at[6]),
    ]

    for cp in small:
        cp.start()
    issue(None, wo_stream(0), skew)
    issue(wq_stream(0), wo_stream(skew), n_qo - skew)
    issue(wq_stream(n_qo - skew), kv_stream(1, 0, False, 0), skew)
    issue_kv(0)

    for cp in small:
        cp.wait()
    x_scr[...] = jnp.concatenate([x_buf[...].astype(jnp.float32), jnp.zeros((M - B, D), jnp.float32)], axis=0)

    wait_all(wq_buf, w_sems.at[0])

    def store_q(j, c0, r):
        r = r.astype(jnp.bfloat16).astype(jnp.float32)
        nh = r.shape[1] // DH
        for b in range(B):
            for t in range(nh):
                q_scr[pl.ds(b * H + j * nh + t, 1), :] = r[b:b + 1, t * DH:(t + 1) * DH]
    x_matmul(wq_buf, store_q, halfway=functools.partial(issue_kv, 1))
    acc_scr[...] = jnp.zeros_like(acc_scr)

    for u in range(2, AH):
        issue_kv(u)
    wait_all(wo_buf, w_sems.at[1])

    scale = DH ** -0.5
    row_s = jax.lax.broadcasted_iota(jnp.int32, (M, span), 0)
    row_o = jax.lax.broadcasted_iota(jnp.int32, (M, DH), 0)
    head_o = row_o // P
    heads_per_seg = wo_buf.shape[1] // DH

    def step(t, c):
        kslot = t % NS
        vslot = t % (NS + 1)
        jj = t % J
        u = t + AH

        @pl.when(u < n_steps)
        def _():
            issue_kv(u)

        @pl.when(u >= n_steps)
        def _():
            issue_gu((u - n_steps) * GU_BURST, GU_BURST)

        @pl.when(jj == 0)
        def _():
            st_scr[0] = jnp.full((M, DH), -jnp.inf, jnp.float32)
            st_scr[1] = jnp.zeros((M, DH), jnp.float32)
            st_scr[2] = jnp.zeros((M, DH), jnp.float32)

        heads = [((t // J) * HG + HEAD0 + a) % NH for a in range(HG)]
        wait_all(k_buf.at[kslot], k_sems.at[kslot])
        q = jnp.broadcast_to(q_scr[pl.ds(heads[0], 1), :], (M, DH))
        for a in range(1, HG):
            q = jnp.where(head_o == a, q_scr[pl.ds(heads[a], 1), :], q)
        q = q.astype(jnp.bfloat16)
        s = _dot(q, k_buf[kslot, 0], _NT)
        for r in range(1, G):
            s = jnp.where(row_s == r, _dot(q, k_buf[kslot, r], _NT), s)
        s = s * scale
        m_old = st_scr[0]
        m_new = jnp.maximum(m_old, jnp.max(s, axis=-1, keepdims=True))
        alpha = jnp.exp(m_old - m_new)
        p = jnp.exp(s - m_new[:, :1])
        st_scr[1] = st_scr[1] * alpha + jnp.sum(p, axis=-1, keepdims=True)
        st_scr[0] = m_new
        pb = p.astype(jnp.bfloat16)

        wait_all(v_buf.at[vslot], v_sems.at[vslot])
        o = _dot(pb, v_buf[vslot, 0])
        for r in range(1, G):
            o = jnp.where(row_o == r, _dot(pb, v_buf[vslot, r]), o)
        st_scr[2] = st_scr[2] * alpha + o

        @pl.when(jj == J - 1)
        def _():
            m, l, o_part = st_scr[0], st_scr[1], st_scr[2]
            acc = acc_scr[...]
            for a in range(HG):
                mine = head_o == a
                m_h = jnp.max(jnp.where(mine, m, -jnp.inf), axis=0, keepdims=True)
                w = jnp.exp(m - m_h)
                l_h = jnp.sum(jnp.where(mine, w * l, 0.0), axis=0, keepdims=True)
                o_h = jnp.sum(jnp.where(mine, w * o_part, 0.0), axis=0, keepdims=True) / l_h
                h = heads[a] % H
                lhs = jnp.where(row_o == heads[a] // H, o_h, 0.0).astype(jnp.bfloat16)
                wo_h = wo_buf[h // heads_per_seg, pl.ds(pl.multiple_of((h % heads_per_seg) * DH, DH), DH), :]
                acc = acc + _dot(lhs, wo_h)
            acc_scr[...] = acc
        return c

    jax.lax.fori_loop(0, n_steps, step, 0)

    issue_gu(AH * GU_BURST, n_gu - skew - AH * GU_BURST)
    issue(wg_stream(n_gu - skew), w_stream(wd_hbm, wd_buf, d_sems.at[0], n_p0 // 2), skew)
    b1, b2, b3 = BURSTS[0], BURSTS[0] + BURSTS[1], sum(BURSTS)
    issue_wd(0, b1)
    wait_all(wg_buf, w_sems.at[2])

    def store_gate(j, c0, r):
        hid_scr[:, pl.ds(c0, r.shape[1])] = r * _sigmoid(r)
    x_matmul(wg_buf, store_gate)
    issue_wd(b1, b2)
    wait_all(wu_buf, w_sems.at[3])

    def store_up(j, c0, r):
        hid_scr[:, pl.ds(c0, r.shape[1])] = hid_scr[:, pl.ds(c0, r.shape[1])] * r
    x_matmul(wu_buf, store_up)
    issue_wd(b2, b3)

    xf = x_scr[...]
    wr = wr_buf[...].astype(jnp.float32).reshape(1, D)
    gw = gw_buf[...].astype(jnp.float32).reshape(1, D)
    r_sel = _sigmoid(jnp.sum(xf * wr, axis=-1, keepdims=True))
    g = _sigmoid(jnp.sum(xf * gw, axis=-1, keepdims=True))
    base = g * acc_scr[...] + (1.0 - g) * (xf + xf * 0.0)
    coef = (1.0 - g) * r_sel

    def down(piece, c0, nc):
        r0 = piece * 128
        y = None
        for sg in range(nseg_d):
            lo = sg * SEG_D + r0
            t = _dot(hid_scr[:, lo:lo + 128].astype(jnp.bfloat16), wd_buf[sg, r0:r0 + 128, c0:c0 + nc])
            y = t if y is None else y + t
        return y

    y = None
    for p in range(3):
        wait_all(wd_buf.at[:, pl.ds(p * 128, 128), :], d_sems.at[p])
        y = down(p, 0, D) if y is None else y + down(p, 0, D)
        if p == 0:
            issue_wd(b3, len(wd_seq))
    c0 = 0
    for t, nc in enumerate(LAST_COLS):
        wait_all(wd_buf.at[:, pl.ds(384, 128), pl.ds(c0, nc)], d_sems.at[3 + t])
        yc = y[:, c0:c0 + nc] + down(3, c0, nc)
        o_ref[:, c0:c0 + nc] = (base[:, c0:c0 + nc] + coef * yc)[:B].astype(o_ref.dtype)
        c0 += nc


@jax.jit
def pallas_gated_mix__mha_block_cached__moe_arch_mod__decode_kernel(
    A_x: jax.Array,
    A_k_cache: jax.Array,
    A_v_cache: jax.Array,
    A_wq: jax.Array,
    A_wo: jax.Array,
    B_x: jax.Array,
    B_w_r: jax.Array,
    B_w_gate: jax.Array,
    B_w_up: jax.Array,
    B_w_down: jax.Array,
    gate_w: jax.Array,
):
    del B_x
    B, _, D = A_x.shape
    _, H, SK, DH = A_k_cache.shape
    F = B_w_gate.shape[1]
    bf, f32 = jnp.bfloat16, jnp.float32
    span = min(SPAN, SK // P // 2)
    kv_shape = (B * H * P, SK // P, DH)
    wq = A_wq.reshape(WSEG, D // WSEG, H * DH)
    wo = A_wo.reshape(WSEG, H * DH // WSEG, D)
    wg = B_w_gate.reshape(WSEG, D // WSEG, F)
    wu = B_w_up.reshape(WSEG, D // WSEG, F)
    wd = B_w_down.reshape(F // SEG_D, SEG_D, D)
    params = dict(vmem_limit_bytes=100 * 1024 * 1024, disable_bounds_checks=True)
    if hasattr(pltpu.CompilerParams, "disable_semaphore_checks"):
        params["disable_semaphore_checks"] = True
    out = pl.pallas_call(
        _kernel,
        in_specs=[pl.BlockSpec(memory_space=pl.ANY)] * 10,
        out_specs=pl.BlockSpec(memory_space=pltpu.VMEM),
        out_shape=jax.ShapeDtypeStruct((B, D), A_x.dtype),
        scratch_shapes=[
            pltpu.VMEM((B, D), bf),
            pltpu.VMEM((D,), bf),
            pltpu.VMEM((D,), bf),
            pltpu.VMEM(wq.shape, bf),
            pltpu.VMEM(wo.shape, bf),
            pltpu.VMEM(wg.shape, bf),
            pltpu.VMEM(wu.shape, bf),
            pltpu.VMEM(wd.shape, bf),
            pltpu.VMEM((NS, G, span, DH), bf),
            pltpu.VMEM((NS + 1, G, span, DH), bf),
            pltpu.VMEM((B * H, DH), f32),
            pltpu.VMEM((M, D), f32),
            pltpu.VMEM((M, F), f32),
            pltpu.VMEM((M, D), f32),
            pltpu.VMEM((3, M, DH), f32),
            pltpu.SemaphoreType.DMA((NS,)),
            pltpu.SemaphoreType.DMA((NS + 1,)),
            pltpu.SemaphoreType.DMA((7,)),
            pltpu.SemaphoreType.DMA((3 + len(LAST_COLS),)),
        ],
        compiler_params=pltpu.CompilerParams(**params),
    )(A_x.reshape(B, D), A_k_cache.reshape(kv_shape), A_v_cache.reshape(kv_shape),
      wq, wo, B_w_r, wg, wu, wd, gate_w)
    return out.reshape(B, 1, D)
```

```python
import functools
import jax
import jax.numpy as jnp
import jax.experimental.pallas as pl
import jax.experimental.pallas.tpu as pltpu

B, D = 4, 1024
H, SK, DH = 32, 8192, 128
F = 3584
M = 8
G = 16
P = 4
HG = G // P
NSEG_D, SEG_D = 7, 512
WC = 256

_NT = (((1,), (1,)), ((), ()))
_NN = (((1,), (0,)), ((), ()))


def _dot(a, b, dims=_NN):
    return jax.lax.dot_general(a, b, dims, preferred_element_type=jnp.float32)


def _sigmoid(x):
    return 1.0 / (1.0 + jnp.exp(-x))


def make(AH=3, span=512, compute=True, skew=24, last_cols=(768, 128, 128), bursts=(76, 62, 62),
         gu_burst=32, solo=2, HEAD0=1, t0first=False, c_loop=True):
    rows = 8
    R = SK // P
    NP = span // rows // 2
    J = R // span
    NH = B * H
    n_seg = NH * P
    n_groups = NH // HG
    n_units = n_groups * 2 * J
    NSL = AH + 2
    first_wrap = (n_groups - 1) * 2 * J
    seg0 = HEAD0 * P
    n_gu = D // 64 * (F // WC)
    n_qo = 256
    n_p0 = 64
    assert HEAD0 in (0, 1) and skew <= NP and NP % 2 == 0 and skew <= n_p0 // 2 and AH * gu_burst + skew <= n_gu and 2 <= AH < first_wrap
    assert R % span == 0 and sum(last_cols) == D

    def kernel(x_hbm, k_hbm, v_hbm, wq_hbm, wo_hbm, wr_hbm, wg_hbm, wu_hbm, wd_hbm, gw_hbm,
               o_ref,
               x_buf, wr_buf, gw_buf, wq_buf, wo_buf, wg_buf, wu_buf, wd_buf,
               kv_buf, q_scr, acc_scr, hid_scr, x_scr, s_scr, o_scr, l_scr,
               kv_sems, w_sems, d_sems):

        def mo(x, m):
            return x if isinstance(x, int) else pl.multiple_of(x, m)

        def kv_stream(thread, u, wrap, off):
            slot = u % NSL
            grp = u // (2 * J)
            is_v = (u // J) % 2
            base = mo((u % J) * span, span)

            def go(s0, d0, ns, r, nr):
                def start(hbm):
                    pltpu.make_async_copy(hbm.at[pl.ds(s0, ns), pl.ds(base + r, nr), :],
                                          kv_buf.at[slot, pl.ds(d0, ns), pl.ds(r, nr), :], kv_sems.at[slot]).start(priority=thread)
                if isinstance(is_v, int):
                    start(v_hbm if is_v else k_hbm)
                else:
                    pl.when(is_v == 0)(functools.partial(start, k_hbm))
                    pl.when(is_v == 1)(functools.partial(start, v_hbm))

            def f(j):
                j = j + off
                if not wrap:
                    go(seg0 + grp * G, 0, G, mo((2 * j + thread) * rows, rows), rows)
                elif thread == 0:
                    go(n_seg - 3 * P, 0, 2 * P, mo(j * 2 * rows, 2 * rows), 2 * rows)
                else:
                    half = j % 2
                    go((1 - half) * (n_seg - P), (2 + half) * P, P, mo((j // 2) * 4 * rows, 4 * rows), 4 * rows)
            return f

        def w_stream(src, dst, sem, thread, off):
            ncb = src.shape[2] // WC

            def f(j):
                j = j + off
                r = mo((j // ncb) * 8, 8)
                c = mo((j % ncb) * WC, 128)
                pltpu.make_async_copy(src.at[:, pl.ds(r, 8), pl.ds(c, WC)],
                                      dst.at[:, pl.ds(r, 8), pl.ds(c, WC)], sem).start(priority=thread)
            return f

        wq_stream = functools.partial(w_stream, wq_hbm, wq_buf, w_sems.at[0], 0)
        wo_stream = functools.partial(w_stream, wo_hbm, wo_buf, w_sems.at[1], 1)
        wg_stream = functools.partial(w_stream, wg_hbm, wg_buf, w_sems.at[2], 0)
        wu_stream = functools.partial(w_stream, wu_hbm, wu_buf, w_sems.at[3], 1)

        def issue(f0, f1, n):
            if n == 0:
                return

            def body(j, c):
                if t0first and f0 is not None:
                    f0(j)
                f1(j)
                if not t0first and f0 is not None:
                    f0(j)
                return c
            jax.lax.fori_loop(0, n, body, 0)

        def issue_kv(u):
            def part_a(wrap):
                issue(kv_stream(0, u, wrap, 0), kv_stream(1, u, wrap, skew), NP - skew)

            def part_b(wrap, next_wrap):
                nxt = wu_stream(0) if next_wrap is None else kv_stream(1, u + 1, next_wrap, 0)
                issue(kv_stream(0, u, wrap, NP - skew), nxt, skew)

            if isinstance(u, int):
                part_a(False)
                part_b(False, False)
                return
            if HEAD0 == 0:
                part_a(False)
                pl.when(u < n_units - 1)(functools.partial(part_b, False, False))
                pl.when(u == n_units - 1)(functools.partial(part_b, False, None))
                return
            pl.when(u < first_wrap)(functools.partial(part_a, False))
            pl.when(u >= first_wrap)(functools.partial(part_a, True))
            pl.when(u < first_wrap - 1)(functools.partial(part_b, False, False))
            pl.when(u == first_wrap - 1)(functools.partial(part_b, False, True))
            pl.when(jnp.logical_and(u >= first_wrap, u < n_units - 1))(functools.partial(part_b, True, True))
            pl.when(u == n_units - 1)(functools.partial(part_b, True, None))

        def issue_gu(off, n):
            issue(wg_stream(off), wu_stream(off + skew), n)

        batches = [(p, p * 128, 0, D) for p in range(3)]
        c0 = 0
        for t, nc in enumerate(last_cols):
            batches.append((3 + t, 384, c0, nc))
            c0 += nc
        L = [[], []]
        for bi, (si, r0, c0, nc) in enumerate(batches):
            w = min(WC, nc)
            assert nc % w == 0
            ds = [(r, c, w, si) for r in range(r0, r0 + 128, 8) for c in range(c0, c0 + nc, w)]
            n0 = 0 if bi >= len(batches) - solo else len(ds) // 2
            L[0] += ds[:n0]
            L[1] += ds[n0:]
        seq = []
        for j in range(max(len(L[0]), len(L[1]))):
            if j + skew < len(L[1]):
                seq.append((1,) + L[1][j + skew])
            if j < len(L[0]):
                seq.append((0,) + L[0][j])

        def issue_wd(lo, hi):
            for t, r, c, w, si in seq[lo:hi]:
                pltpu.make_async_copy(wd_hbm.at[:, pl.ds(r, 8), pl.ds(c, w)], wd_buf.at[:, pl.ds(r, 8), pl.ds(c, w)],
                                      d_sems.at[si]).start(priority=t)

        def wait_all(buf, sem):
            pltpu.make_async_copy(buf, buf, sem).wait()

        def x_matmul(w_buf, store, cb=512, mids=()):
            s, r, c = w_buf.shape

            def body(j, carry):
                for at, fn in mids:
                    pl.when(j == at)(fn)
                c0 = pl.multiple_of(j * cb, 128)
                w = w_buf[:, :, pl.ds(c0, cb)].reshape(s * r, cb)
                store(j, c0, _dot(x_scr[...].astype(jnp.bfloat16), w))
                return carry
            jax.lax.fori_loop(0, c // cb, body, 0)

        small = [
            pltpu.make_async_copy(x_hbm, x_buf, w_sems.at[4]),
            pltpu.make_async_copy(wr_hbm, wr_buf, w_sems.at[5]),
            pltpu.make_async_copy(gw_hbm, gw_buf, w_sems.at[6]),
        ]

        for cp in small:
            cp.start()
        issue(None, wo_stream(0), skew)
        issue(wq_stream(0), wo_stream(skew), n_qo - skew)
        issue(wq_stream(n_qo - skew), kv_stream(1, 0, False, 0), skew)
        issue_kv(0)
        issue_kv(1)

        for cp in small:
            cp.wait()
        x_scr[...] = jnp.concatenate([x_buf[...].astype(jnp.float32), jnp.zeros((M - B, D), jnp.float32)], axis=0)
        wait_all(wq_buf, w_sems.at[0])

        def store_q(j, c0, r):
            r = r.astype(jnp.bfloat16).astype(jnp.float32)
            nh = r.shape[1] // DH
            for b in range(B):
                for t in range(nh):
                    q_scr[pl.ds(b * H + j * nh + t, 1), :] = r[b:b + 1, t * DH:(t + 1) * DH]
        nxt = 2
        if compute:
            if AH > 2:
                x_matmul(wq_buf, store_q, mids=((4, functools.partial(issue_kv, 2)),))
                nxt = 3
            else:
                x_matmul(wq_buf, store_q)
        acc_scr[...] = jnp.zeros_like(acc_scr)
        for u in range(nxt, AH):
            issue_kv(u)
        wait_all(wo_buf, w_sems.at[1])

        scale = DH ** -0.5
        row_s = jax.lax.broadcasted_iota(jnp.int32, (M, span), 0)
        row_o = jax.lax.broadcasted_iota(jnp.int32, (M, DH), 0)
        lo_o = row_o < P
        NHALF = G // M

        def step(t, c):
            slot = t % NSL
            grp = t // (2 * J)
            is_v = (t // J) % 2
            jj = t % J
            u = t + AH

            @pl.when(u < n_units)
            def _():
                issue_kv(u)

            @pl.when(u >= n_units)
            def _():
                issue_gu((u - n_units) * gu_burst, gu_burst)

            heads = [(grp * HG + HEAD0 + a) % NH for a in range(HG)]
            col = pl.multiple_of(jj * span, span)
            wait_all(kv_buf.at[slot], kv_sems.at[slot])
            if not (compute and c_loop):
                return c

            @pl.when(is_v == 0)
            def _():
                for hf in range(NHALF):
                    q = jnp.where(lo_o, q_scr[pl.ds(heads[2 * hf], 1), :], q_scr[pl.ds(heads[2 * hf + 1], 1), :]).astype(jnp.bfloat16)
                    s = _dot(q, kv_buf[slot, hf * M], _NT)
                    for r in range(1, M):
                        s = jnp.where(row_s == r, _dot(q, kv_buf[slot, hf * M + r], _NT), s)
                    s_scr[hf, :, pl.ds(col, span)] = s * scale

                @pl.when(jj == J - 1)
                def _():
                    for hf in range(NHALF):
                        s = s_scr[hf]
                        m = jnp.broadcast_to(jnp.max(s, axis=-1, keepdims=True), (M, DH))
                        m_lo = jnp.max(jnp.where(lo_o, m, -jnp.inf), axis=0, keepdims=True)
                        m_hi = jnp.max(jnp.where(lo_o, -jnp.inf, m), axis=0, keepdims=True)
                        m_h = jnp.where(lo_o, m_lo, m_hi)
                        p = jnp.exp(s - m_h[:, :1])
                        s_scr[hf] = p
                        l_scr[hf] = jnp.broadcast_to(jnp.sum(p, axis=-1, keepdims=True), (M, DH))
                        o_scr[hf] = jnp.zeros((M, DH), jnp.float32)

            @pl.when(is_v == 1)
            def _():
                for hf in range(NHALF):
                    pb = s_scr[hf, :, pl.ds(col, span)].astype(jnp.bfloat16)
                    o = _dot(pb, kv_buf[slot, hf * M])
                    for r in range(1, M):
                        o = jnp.where(row_o == r, _dot(pb, kv_buf[slot, hf * M + r]), o)
                    o_scr[hf] += o

                @pl.when(jj == J - 1)
                def _():
                    acc = acc_scr[...]
                    for a in range(HG):
                        mine = lo_o if a % 2 == 0 else jnp.logical_not(lo_o)
                        l_h = jnp.sum(jnp.where(mine, l_scr[a // 2], 0.0), axis=0, keepdims=True)
                        o_h = jnp.sum(jnp.where(mine, o_scr[a // 2], 0.0), axis=0, keepdims=True) / l_h
                        h = heads[a] % H
                        lhs = jnp.where(row_o == heads[a] // H, o_h, 0.0).astype(jnp.bfloat16)
                        acc = acc + _dot(lhs, wo_buf[h // 4, pl.ds(pl.multiple_of((h % 4) * DH, DH), DH), :])
                    acc_scr[...] = acc
            return c

        jax.lax.fori_loop(0, n_units, step, 0)

        issue_gu(AH * gu_burst, n_gu - skew - AH * gu_burst)
        issue(wg_stream(n_gu - skew), w_stream(wd_hbm, wd_buf, d_sems.at[0], 1, n_p0 // 2), skew)
        b1, b2, b3 = bursts[0], bursts[0] + bursts[1], sum(bursts)
        issue_wd(0, b1)
        wait_all(wg_buf, w_sems.at[2])
        if compute:
            def store_gate(j, c0, r):
                hid_scr[:, pl.ds(c0, r.shape[1])] = r * _sigmoid(r)
            x_matmul(wg_buf, store_gate)
        issue_wd(b1, b2)
        wait_all(wu_buf, w_sems.at[3])
        if compute:
            def store_up(j, c0, r):
                hid_scr[:, pl.ds(c0, r.shape[1])] = hid_scr[:, pl.ds(c0, r.shape[1])] * r
            x_matmul(wu_buf, store_up)
        issue_wd(b2, b3)

        xf = x_scr[...]
        wr = wr_buf[...].astype(jnp.float32).reshape(1, D)
        gw = gw_buf[...].astype(jnp.float32).reshape(1, D)
        r_sel = _sigmoid(jnp.sum(xf * wr, axis=-1, keepdims=True))
        g = _sigmoid(jnp.sum(xf * gw, axis=-1, keepdims=True))
        base = g * acc_scr[...] + (1.0 - g) * (xf + xf * 0.0)
        coef = (1.0 - g) * r_sel

        def down(piece, c0, nc):
            r0 = piece * 128
            y = None
            for sg in range(NSEG_D):
                lo = sg * SEG_D + r0
                t = _dot(hid_scr[:, lo:lo + 128].astype(jnp.bfloat16), wd_buf[sg, r0:r0 + 128, c0:c0 + nc])
                y = t if y is None else y + t
            return y

        y = jnp.zeros((M, D), jnp.float32)
        for p in range(3):
            wait_all(wd_buf.at[:, pl.ds(p * 128, 128), :], d_sems.at[p])
            if compute:
                y = y + down(p, 0, D)
            if p == 0:
                issue_wd(b3, len(seq))
        c0 = 0
        for t, nc in enumerate(last_cols):
            wait_all(wd_buf.at[:, pl.ds(384, 128), pl.ds(c0, nc)], d_sems.at[3 + t])
            yc = y[:, c0:c0 + nc]
            if compute:
                yc = yc + down(3, c0, nc)
            o_ref[:, c0:c0 + nc] = (base[:, c0:c0 + nc] + coef * yc)[:B].astype(o_ref.dtype)
            c0 += nc

    @jax.jit
    def fn(A_x, A_k_cache, A_v_cache, A_wq, A_wo, B_x, B_w_r, B_w_gate, B_w_up, B_w_down, gate_w):
        bf, f32 = jnp.bfloat16, jnp.float32
        wq = A_wq.reshape(8, D // 8, H * DH)
        wg = B_w_gate.reshape(8, D // 8, F)
        wu = B_w_up.reshape(8, D // 8, F)
        wo = A_wo.reshape(8, 512, D)
        wd = B_w_down.reshape(NSEG_D, SEG_D, D)
        kv_shape = (n_seg, R, DH)
        out = pl.pallas_call(
            kernel,
            in_specs=[pl.BlockSpec(memory_space=pl.ANY)] * 10,
            out_specs=pl.BlockSpec(memory_space=pltpu.VMEM),
            out_shape=jax.ShapeDtypeStruct((B, D), A_x.dtype),
            scratch_shapes=[
                pltpu.VMEM((B, D), bf),
                pltpu.VMEM((D,), bf),
                pltpu.VMEM((D,), bf),
                pltpu.VMEM(wq.shape, bf),
                pltpu.VMEM(wo.shape, bf),
                pltpu.VMEM(wg.shape, bf),
                pltpu.VMEM(wu.shape, bf),
                pltpu.VMEM(wd.shape, bf),
                pltpu.VMEM((NSL, G, span, DH), bf),
                pltpu.VMEM((NH, DH), f32),
                pltpu.VMEM((M, D), f32),
                pltpu.VMEM((M, F), f32),
                pltpu.VMEM((M, D), f32),
                pltpu.VMEM((G // M, M, R), f32),
                pltpu.VMEM((G // M, M, DH), f32),
                pltpu.VMEM((G // M, M, DH), f32),
                pltpu.SemaphoreType.DMA((NSL,)),
                pltpu.SemaphoreType.DMA((7,)),
                pltpu.SemaphoreType.DMA((3 + len(last_cols),)),
            ],
            compiler_params=pltpu.CompilerParams(
                vmem_limit_bytes=100 * 1024 * 1024,
                disable_bounds_checks=True,
                disable_semaphore_checks=True,
            ),
        )(A_x.reshape(B, D), A_k_cache.reshape(kv_shape), A_v_cache.reshape(kv_shape),
          wq, wo, B_w_r, wg, wu, wd, gate_w)
        return out.reshape(B, 1, D)
    return fn


_IMPL = make()


@jax.jit
def pallas_gated_mix__mha_block_cached__moe_arch_mod__decode_kernel(
    A_x: jax.Array,
    A_k_cache: jax.Array,
    A_v_cache: jax.Array,
    A_wq: jax.Array,
    A_wo: jax.Array,
    B_x: jax.Array,
    B_w_r: jax.Array,
    B_w_gate: jax.Array,
    B_w_up: jax.Array,
    B_w_down: jax.Array,
    gate_w: jax.Array,
):
    return _IMPL(A_x, A_k_cache, A_v_cache, A_wq, A_wo, B_x, B_w_r, B_w_gate, B_w_up, B_w_down, gate_w)
```

```python
import functools

import jax
import jax.numpy as jnp
import jax.experimental.pallas as pl
import jax.experimental.pallas.tpu as pltpu

M = 8
G = 16
P = 4
HG = G // P
HEAD0 = 1
ROWS = 8
SPAN = 512
AH = 3
NSL = AH + 2
SKEW = 24
WSEG = 8
WC = 256
SEG_D = 512
GU_BURST = 32
LAST_COLS = (768, 128, 128)
SOLO = 2
BURSTS = (76, 62, 62)

_NT = (((1,), (1,)), ((), ()))
_NN = (((1,), (0,)), ((), ()))


def _dot(a, b, dims=_NN):
    return jax.lax.dot_general(a, b, dims, preferred_element_type=jnp.float32)


def _sigmoid(x):
    return 1.0 / (1.0 + jnp.exp(-x))


def _mo(x, m):
    return x if isinstance(x, int) else pl.multiple_of(x, m)


def _w_down_schedule(d, skew):
    batches = [(p, p * 128, 0, d) for p in range(3)]
    c0 = 0
    for t, nc in enumerate(LAST_COLS):
        batches.append((3 + t, 384, c0, nc))
        c0 += nc
    assert c0 == d
    lists = [[], []]
    for bi, (si, r0, c0, nc) in enumerate(batches):
        w = min(WC, nc)
        assert nc % w == 0
        ds = [(r, c, w, si) for r in range(r0, r0 + 128, 8) for c in range(c0, c0 + nc, w)]
        n0 = 0 if bi >= len(batches) - SOLO else len(ds) // 2
        lists[0] += ds[:n0]
        lists[1] += ds[n0:]
    seq = []
    for j in range(max(len(lists[0]), len(lists[1]))):
        if j + skew < len(lists[1]):
            seq.append((1,) + lists[1][j + skew])
        if j < len(lists[0]):
            seq.append((0,) + lists[0][j])
    return seq


def _kernel(x_hbm, k_hbm, v_hbm, wq_hbm, wo_hbm, wr_hbm, wg_hbm, wu_hbm, wd_hbm, gw_hbm,
            o_ref,
            x_buf, wr_buf, gw_buf, wq_buf, wo_buf, wg_buf, wu_buf, wd_buf,
            kv_buf, q_scr, acc_scr, hid_scr, x_scr, s_scr, o_scr, l_scr,
            kv_sems, w_sems, d_sems):
    B, D = x_buf.shape
    n_seg, R, DH = k_hbm.shape
    NH = n_seg // P
    H = NH // B
    span = kv_buf.shape[2]
    nseg_d = wd_buf.shape[0]
    NP = span // ROWS // 2
    J = R // span
    n_groups = NH // HG
    n_units = n_groups * 2 * J
    first_wrap = (n_groups - 1) * 2 * J
    skew = min(SKEW, NP - 2)
    n_qo = wq_buf.shape[1] // 8 * (wq_buf.shape[2] // WC)
    n_gu = wg_buf.shape[1] // 8 * (wg_buf.shape[2] // WC)
    n_p0 = 128 // 8 * (D // WC)
    assert n_qo == wo_buf.shape[1] // 8 * (wo_buf.shape[2] // WC)
    assert HEAD0 == 1 and HG == 4 and G == 2 * M and NP % 2 == 0 and R % span == 0 and 3 <= AH < first_wrap
    assert skew <= n_p0 // 2 and AH * GU_BURST + skew <= n_gu and wd_buf.shape[1] == SEG_D == 512

    def kv_stream(thread, u, wrap, off):
        slot = u % NSL
        is_v = (u // J) % 2
        base = _mo((u % J) * span, span)

        def go(s0, d0, ns, r, nr):
            def start(hbm):
                pltpu.make_async_copy(hbm.at[pl.ds(s0, ns), pl.ds(base + r, nr), :],
                                      kv_buf.at[slot, pl.ds(d0, ns), pl.ds(r, nr), :],
                                      kv_sems.at[slot]).start(priority=thread)
            if isinstance(is_v, int):
                start(v_hbm if is_v else k_hbm)
            else:
                pl.when(is_v == 0)(functools.partial(start, k_hbm))
                pl.when(is_v == 1)(functools.partial(start, v_hbm))

        def f(j):
            j = j + off
            if not wrap:
                go(HEAD0 * P + (u // (2 * J)) * G, 0, G, _mo((2 * j + thread) * ROWS, ROWS), ROWS)
            elif thread == 0:
                go(n_seg - 3 * P, 0, 2 * P, _mo(j * 2 * ROWS, 2 * ROWS), 2 * ROWS)
            else:
                half = j % 2
                go((1 - half) * (n_seg - P), (2 + half) * P, P, _mo((j // 2) * 4 * ROWS, 4 * ROWS), 4 * ROWS)
        return f

    def w_stream(src, dst, sem, thread, off):
        ncb = src.shape[2] // WC

        def f(j):
            j = j + off
            r = _mo((j // ncb) * 8, 8)
            c = _mo((j % ncb) * WC, 128)
            pltpu.make_async_copy(src.at[:, pl.ds(r, 8), pl.ds(c, WC)],
                                  dst.at[:, pl.ds(r, 8), pl.ds(c, WC)], sem).start(priority=thread)
        return f

    wq_stream = functools.partial(w_stream, wq_hbm, wq_buf, w_sems.at[0], 0)
    wo_stream = functools.partial(w_stream, wo_hbm, wo_buf, w_sems.at[1], 1)
    wg_stream = functools.partial(w_stream, wg_hbm, wg_buf, w_sems.at[2], 0)
    wu_stream = functools.partial(w_stream, wu_hbm, wu_buf, w_sems.at[3], 1)

    def issue(f0, f1, n):
        def body(j, c):
            f1(j)
            if f0 is not None:
                f0(j)
            return c
        jax.lax.fori_loop(0, n, body, 0)

    def issue_kv(u):
        def part_a(wrap):
            issue(kv_stream(0, u, wrap, 0), kv_stream(1, u, wrap, skew), NP - skew)

        def part_b(wrap, next_wrap):
            nxt = wu_stream(0) if next_wrap is None else kv_stream(1, u + 1, next_wrap, 0)
            issue(kv_stream(0, u, wrap, NP - skew), nxt, skew)

        if isinstance(u, int):
            part_a(False)
            part_b(False, False)
            return
        pl.when(u < first_wrap)(functools.partial(part_a, False))
        pl.when(u >= first_wrap)(functools.partial(part_a, True))
        pl.when(u < first_wrap - 1)(functools.partial(part_b, False, False))
        pl.when(u == first_wrap - 1)(functools.partial(part_b, False, True))
        pl.when(jnp.logical_and(u >= first_wrap, u < n_units - 1))(functools.partial(part_b, True, True))
        pl.when(u == n_units - 1)(functools.partial(part_b, True, None))

    def issue_gu(off, n):
        issue(wg_stream(off), wu_stream(off + skew), n)

    wd_seq = _w_down_schedule(D, skew)

    def issue_wd(lo, hi):
        for t, r, c, w, si in wd_seq[lo:hi]:
            pltpu.make_async_copy(wd_hbm.at[:, pl.ds(r, 8), pl.ds(c, w)], wd_buf.at[:, pl.ds(r, 8), pl.ds(c, w)],
                                  d_sems.at[si]).start(priority=t)

    def wait_all(buf, sem):
        pltpu.make_async_copy(buf, buf, sem).wait()

    def x_matmul(w_buf, store, cb=512, halfway=None):
        s, r, c = w_buf.shape

        def body(j, carry):
            if halfway is not None:
                pl.when(j == c // cb // 2)(halfway)
            c0 = pl.multiple_of(j * cb, 128)
            w = w_buf[:, :, pl.ds(c0, cb)].reshape(s * r, cb)
            store(j, c0, _dot(x_scr[...].astype(jnp.bfloat16), w))
            return carry
        jax.lax.fori_loop(0, c // cb, body, 0)

    small = [
        pltpu.make_async_copy(x_hbm, x_buf, w_sems.at[4]),
        pltpu.make_async_copy(wr_hbm, wr_buf, w_sems.at[5]),
        pltpu.make_async_copy(gw_hbm, gw_buf, w_sems.at[6]),
    ]

    for cp in small:
        cp.start()
    issue(None, wo_stream(0), skew)
    issue(wq_stream(0), wo_stream(skew), n_qo - skew)
    issue(wq_stream(n_qo - skew), kv_stream(1, 0, False, 0), skew)
    issue_kv(0)
    issue_kv(1)

    for cp in small:
        cp.wait()
    x_scr[...] = jnp.concatenate([x_buf[...].astype(jnp.float32), jnp.zeros((M - B, D), jnp.float32)], axis=0)
    wait_all(wq_buf, w_sems.at[0])

    def store_q(j, c0, r):
        r = r.astype(jnp.bfloat16).astype(jnp.float32)
        nh = r.shape[1] // DH
        for b in range(B):
            for t in range(nh):
                q_scr[pl.ds(b * H + j * nh + t, 1), :] = r[b:b + 1, t * DH:(t + 1) * DH]
    x_matmul(wq_buf, store_q, halfway=functools.partial(issue_kv, 2))
    acc_scr[...] = jnp.zeros_like(acc_scr)
    for u in range(3, AH):
        issue_kv(u)
    wait_all(wo_buf, w_sems.at[1])

    scale = DH ** -0.5
    row_s = jax.lax.broadcasted_iota(jnp.int32, (M, span), 0)
    row_o = jax.lax.broadcasted_iota(jnp.int32, (M, DH), 0)
    first = row_o < P
    heads_per_seg = wo_buf.shape[1] // DH

    def step(t, c):
        slot = t % NSL
        is_v = (t // J) % 2
        jj = t % J
        u = t + AH

        @pl.when(u < n_units)
        def _():
            issue_kv(u)

        @pl.when(u >= n_units)
        def _():
            issue_gu((u - n_units) * GU_BURST, GU_BURST)

        heads = [((t // (2 * J)) * HG + HEAD0 + a) % NH for a in range(HG)]
        col = pl.multiple_of(jj * span, span)
        wait_all(kv_buf.at[slot], kv_sems.at[slot])

        @pl.when(is_v == 0)
        def _():
            for hf in range(2):
                q = jnp.where(first, q_scr[pl.ds(heads[2 * hf], 1), :], q_scr[pl.ds(heads[2 * hf + 1], 1), :])
                q = q.astype(jnp.bfloat16)
                s = _dot(q, kv_buf[slot, hf * M], _NT)
                for r in range(1, M):
                    s = jnp.where(row_s == r, _dot(q, kv_buf[slot, hf * M + r], _NT), s)
                s_scr[hf, :, pl.ds(col, span)] = s * scale

            @pl.when(jj == J - 1)
            def _():
                for hf in range(2):
                    s = s_scr[hf]
                    m = jnp.broadcast_to(jnp.max(s, axis=-1, keepdims=True), (M, DH))
                    m_a = jnp.max(jnp.where(first, m, -jnp.inf), axis=0, keepdims=True)
                    m_b = jnp.max(jnp.where(first, -jnp.inf, m), axis=0, keepdims=True)
                    p = jnp.exp(s - jnp.where(first, m_a, m_b)[:, :1])
                    s_scr[hf] = p
                    l_scr[hf] = jnp.broadcast_to(jnp.sum(p, axis=-1, keepdims=True), (M, DH))
                    o_scr[hf] = jnp.zeros((M, DH), jnp.float32)

        @pl.when(is_v == 1)
        def _():
            for hf in range(2):
                pb = s_scr[hf, :, pl.ds(col, span)].astype(jnp.bfloat16)
                o = _dot(pb, kv_buf[slot, hf * M])
                for r in range(1, M):
                    o = jnp.where(row_o == r, _dot(pb, kv_buf[slot, hf * M + r]), o)
                o_scr[hf] += o

            @pl.when(jj == J - 1)
            def _():
                acc = acc_scr[...]
                for a in range(HG):
                    mine = first if a % 2 == 0 else jnp.logical_not(first)
                    l_h = jnp.sum(jnp.where(mine, l_scr[a // 2], 0.0), axis=0, keepdims=True)
                    o_h = jnp.sum(jnp.where(mine, o_scr[a // 2], 0.0), axis=0, keepdims=True) / l_h
                    h = heads[a] % H
                    lhs = jnp.where(row_o == heads[a] // H, o_h, 0.0).astype(jnp.bfloat16)
                    wo_h = wo_buf[h // heads_per_seg, pl.ds(pl.multiple_of((h % heads_per_seg) * DH, DH), DH), :]
                    acc = acc + _dot(lhs, wo_h)
                acc_scr[...] = acc
        return c

    jax.lax.fori_loop(0, n_units, step, 0)

    issue_gu(AH * GU_BURST, n_gu - skew - AH * GU_BURST)
    issue(wg_stream(n_gu - skew), w_stream(wd_hbm, wd_buf, d_sems.at[0], 1, n_p0 // 2), skew)
    b1, b2, b3 = BURSTS[0], BURSTS[0] + BURSTS[1], sum(BURSTS)
    issue_wd(0, b1)
    wait_all(wg_buf, w_sems.at[2])

    def store_gate(j, c0, r):
        hid_scr[:, pl.ds(c0, r.shape[1])] = r * _sigmoid(r)
    x_matmul(wg_buf, store_gate)
    issue_wd(b1, b2)
    wait_all(wu_buf, w_sems.at[3])

    def store_up(j, c0, r):
        hid_scr[:, pl.ds(c0, r.shape[1])] = hid_scr[:, pl.ds(c0, r.shape[1])] * r
    x_matmul(wu_buf, store_up)
    issue_wd(b2, b3)

    xf = x_scr[...]
    wr = wr_buf[...].astype(jnp.float32).reshape(1, D)
    gw = gw_buf[...].astype(jnp.float32).reshape(1, D)
    r_sel = _sigmoid(jnp.sum(xf * wr, axis=-1, keepdims=True))
    g = _sigmoid(jnp.sum(xf * gw, axis=-1, keepdims=True))
    base = g * acc_scr[...] + (1.0 - g) * (xf + xf * 0.0)
    coef = (1.0 - g) * r_sel

    def down(piece, c0, nc):
        r0 = piece * 128
        y = None
        for sg in range(nseg_d):
            lo = sg * SEG_D + r0
            t = _dot(hid_scr[:, lo:lo + 128].astype(jnp.bfloat16), wd_buf[sg, r0:r0 + 128, c0:c0 + nc])
            y = t if y is None else y + t
        return y

    y = None
    for p in range(3):
        wait_all(wd_buf.at[:, pl.ds(p * 128, 128), :], d_sems.at[p])
        y = down(p, 0, D) if y is None else y + down(p, 0, D)
        if p == 0:
            issue_wd(b3, len(wd_seq))
    c0 = 0
    for t, nc in enumerate(LAST_COLS):
        wait_all(wd_buf.at[:, pl.ds(384, 128), pl.ds(c0, nc)], d_sems.at[3 + t])
        yc = y[:, c0:c0 + nc] + down(3, c0, nc)
        o_ref[:, c0:c0 + nc] = (base[:, c0:c0 + nc] + coef * yc)[:B].astype(o_ref.dtype)
        c0 += nc


@jax.jit
def pallas_gated_mix__mha_block_cached__moe_arch_mod__decode_kernel(
    A_x: jax.Array,
    A_k_cache: jax.Array,
    A_v_cache: jax.Array,
    A_wq: jax.Array,
    A_wo: jax.Array,
    B_x: jax.Array,
    B_w_r: jax.Array,
    B_w_gate: jax.Array,
    B_w_up: jax.Array,
    B_w_down: jax.Array,
    gate_w: jax.Array,
):
    del B_x
    B, _, D = A_x.shape
    _, H, SK, DH = A_k_cache.shape
    F = B_w_gate.shape[1]
    bf, f32 = jnp.bfloat16, jnp.float32
    R = SK // P
    span = min(SPAN, R // 2)
    kv_shape = (B * H * P, R, DH)
    wq = A_wq.reshape(WSEG, D // WSEG, H * DH)
    wo = A_wo.reshape(WSEG, H * DH // WSEG, D)
    wg = B_w_gate.reshape(WSEG, D // WSEG, F)
    wu = B_w_up.reshape(WSEG, D // WSEG, F)
    wd = B_w_down.reshape(F // SEG_D, SEG_D, D)
    params = dict(vmem_limit_bytes=100 * 1024 * 1024, disable_bounds_checks=True)
    if hasattr(pltpu.CompilerParams, "disable_semaphore_checks"):
        params["disable_semaphore_checks"] = True
    out = pl.pallas_call(
        _kernel,
        in_specs=[pl.BlockSpec(memory_space=pl.ANY)] * 10,
        out_specs=pl.BlockSpec(memory_space=pltpu.VMEM),
        out_shape=jax.ShapeDtypeStruct((B, D), A_x.dtype),
        scratch_shapes=[
            pltpu.VMEM((B, D), bf),
            pltpu.VMEM((D,), bf),
            pltpu.VMEM((D,), bf),
            pltpu.VMEM(wq.shape, bf),
            pltpu.VMEM(wo.shape, bf),
            pltpu.VMEM(wg.shape, bf),
            pltpu.VMEM(wu.shape, bf),
            pltpu.VMEM(wd.shape, bf),
            pltpu.VMEM((NSL, G, span, DH), bf),
            pltpu.VMEM((B * H, DH), f32),
            pltpu.VMEM((M, D), f32),
            pltpu.VMEM((M, F), f32),
            pltpu.VMEM((M, D), f32),
            pltpu.VMEM((2, M, R), f32),
            pltpu.VMEM((2, M, DH), f32),
            pltpu.VMEM((2, M, DH), f32),
            pltpu.SemaphoreType.DMA((NSL,)),
            pltpu.SemaphoreType.DMA((7,)),
            pltpu.SemaphoreType.DMA((3 + len(LAST_COLS),)),
        ],
        compiler_params=pltpu.CompilerParams(**params),
    )(A_x.reshape(B, D), A_k_cache.reshape(kv_shape), A_v_cache.reshape(kv_shape),
      wq, wo, B_w_r, wg, wu, wd, gate_w)
    return out.reshape(B, 1, D)
```
